```python
import os as _os
_os.environ.setdefault("JAX_PLATFORMS", "cpu")
import jax
import jax.numpy as jnp

def _softmax(x, axis=-1):
    return jax.nn.softmax(x, axis=axis)
def _gelu(x):
    return jax.nn.gelu(x, approximate=True)
def _silu(x):
    return jax.nn.silu(x)
def _sigmoid(x):
    return jax.nn.sigmoid(x)
def _layernorm(x, axis=-1, eps=1e-5):
    m = jnp.mean(x, axis=axis, keepdims=True)
    v = jnp.var(x, axis=axis, keepdims=True)
    return (x - m) / jnp.sqrt(v + eps)
def _scatter_add(tgt, idx, src, axis=0):
    return tgt.at[idx].add(src)
def _segment_sum(src, seg, n):
    return jax.ops.segment_sum(src, seg, n)
class _Rng:
    def __init__(self, key):
        self._k = key
    def _next(self):
        self._k, sub = jax.random.split(self._k)
        return sub
    def normal(self, shape):
        return jax.random.normal(self._next(), shape, dtype=jnp.bfloat16)
    def randint(self, lo, hi, shape):
        return jax.random.randint(self._next(), shape, lo, hi, dtype=jnp.int32)
    def uniform(self, shape, lo=0.0, hi=1.0):
        return jax.random.uniform(self._next(), shape, jnp.bfloat16, lo, hi)
    def permutation(self, n):
        return jax.random.permutation(self._next(), n)


kernel_name = 'gated_mix__grouped_kv_mqa__swiglu_ffn__prompt'

def setup_inputs():
    _rng = _Rng(jax.random.key(int.from_bytes(__import__("os").urandom(4), "little")))
    _w = (lambda a: (lambda t: t.astype(jnp.bfloat16) if jnp.issubdtype(t.dtype, jnp.floating) else t)(jnp.asarray(a)))
    def _A_setup():
        B, S, D, H = 1, 2048, 512, 32
        Dh = D // H
        return {
            "x": _w((lambda *s: _rng.normal(s) * 0.05)(B, S, D)),
            "wq": _w((lambda *s: _rng.normal(s) * 0.4)(D, H * Dh)),
            "wk": _w((lambda *s: _rng.normal(s) * 0.4)(D, Dh)),
            "wv": _w((lambda *s: _rng.normal(s) * 0.05)(D, Dh)),
            "wo": _w((lambda *s: _rng.normal(s) * 0.05)(H * Dh, D)),
        }
    _A_in = _A_setup()

    def _B_setup():
        B, S, D, F = 1, 2048, 512, 1792
        return {
            "x": _w((lambda *s: _rng.normal(s) * 0.05)(B, S, D)),
            "w_gate": _w((lambda *s: _rng.normal(s) * 0.05)(D, F)),
            "w_up": _w((lambda *s: _rng.normal(s) * 0.05)(D, F)),
            "w_down": _w((lambda *s: _rng.normal(s) * 0.05)(F, D)),
        }
    _B_in = _B_setup()

    return {
        "A_x": _A_in["x"],
        "A_wq": _A_in["wq"],
        "A_wk": _A_in["wk"],
        "A_wv": _A_in["wv"],
        "A_wo": _A_in["wo"],
        "B_x": _B_in["x"],
        "B_w_gate": _B_in["w_gate"],
        "B_w_up": _B_in["w_up"],
        "B_w_down": _B_in["w_down"],
        "gate_w": _w((lambda *s: _rng.normal(s) * 0.05)(512) * 16.0),
    }

def reference(A_x, A_wq, A_wk, A_wv, A_wo, B_x, B_w_gate, B_w_up, B_w_down, gate_w):
    def _A_ref(x, wq, wk, wv, wo):
        B, S, D = x.shape
        H = 32
        Dh = D // H
        q = (lambda x, *d: x.transpose(*d))((x @ wq).reshape(B, S, H, Dh), 0, 2, 1, 3)
        k = x @ wk
        v = x @ wv
        scores = jnp.einsum("bhqd,bkd->bhqk", q, k) * (Dh ** -0.5)
        p = _softmax(scores, axis=-1)
        o = jnp.einsum("bhqk,bkd->bhqd", p, v)
        return (lambda x, *d: x.transpose(*d))(o, 0, 2, 1, 3).reshape(B, S, H * Dh) @ wo

    def _B_ref(x, w_gate, w_up, w_down):
        g = _silu(x @ w_gate)
        u = x @ w_up
        return (g * u) @ w_down

    x = A_x
    g = _sigmoid((x * gate_w).sum(-1, keepdims=True))
    a = _A_ref(x, A_wq, A_wk, A_wv, A_wo)
    b = _B_ref(x, B_w_gate, B_w_up, B_w_down)
    return g * a + (1 - g) * b
```

```python
import math
import jax
import jax.numpy as jnp
from jax import lax
from jax.experimental import pallas as pl
from jax.experimental.pallas import tpu as pltpu

S = 2048; D = 512; H = 32; DH = 16; F = 1792
TQ = 512
CK = 128
NCK = S // CK
NCT = TQ // 128
SKEW = 2
HPB = 4
FC = 256
DEPD = 2
G = 5
XV = 8 * G * (NCK // NCT)
LAG = NCK + SKEW
NQ = 8
TOFF = -2
TSPAN = 14
QSCALE = (DH ** -0.5) * math.log2(math.e)
f32 = jnp.float32; bf16 = jnp.bfloat16; u32 = jnp.uint32
_n16 = (S - XV) // 16
ROWS = [16 * ((_n16 * (c + 1)) // NCK - (_n16 * c) // NCK) for c in range(NCK)]
STARTS = [XV + sum(ROWS[:c]) for c in range(NCK)]


def kernel(x_ref, wq_ref, wkt_ref, wvt_ref, gw_ref, wo_hbm, wg_hbm, wu_hbm, wd_hbm, o_ref,
           wkv_scr, kv_scr, vt_scr, wqt_scr, qt_scr, ot_scr, sA, sB, wo_ref, wg_ref, wu_ref, wd_ref,
           kb_scr, qtf_scr, qbA, qbB, sems):
    i = pl.program_id(0)

    def copies():
        return [pltpu.make_async_copy(src, dst, sems.at[n])
                for n, (src, dst) in enumerate(((wo_hbm, wo_ref), (wg_hbm, wg_ref), (wu_hbm, wu_ref), (wd_hbm, wd_ref)))]

    @pl.when(i == 0)
    def _():
        for c in copies():
            c.start()
        wkv_scr[0:DH, :] = wkt_ref[...]
        wkv_scr[DH:2 * DH, :] = wvt_ref[...]
        wkv_scr[2 * DH:, :] = jnp.zeros((128 - 2 * DH, D), bf16)
        kv = lax.dot_general(x_ref[...], wkv_scr[...], (((1,), (1,)), ((), ())), preferred_element_type=f32)
        kvb = kv.astype(bf16)
        kv_scr[...] = pltpu.bitcast(kvb, u32)
        vt_scr[...] = pltpu.bitcast(kv.T[DH:2 * DH, :].astype(bf16), u32)
        wqt_scr[...] = wq_ref[...].astype(f32).T.astype(bf16)
        if G:
            rows = kvb[:XV, :].astype(f32)
            for d in range(DH):
                kb_scr[d] = jnp.broadcast_to(rows[:, d:d + 1], (XV, 128))

    row0 = pl.multiple_of(i * TQ, TQ)
    xq = x_ref[pl.ds(row0, TQ), :]
    qt = lax.dot_general(wqt_scr[...], xq, (((1,), (1,)), ((), ())), preferred_element_type=f32)
    qtb = (qt * QSCALE).astype(bf16)
    qt_scr[...] = pltpu.bitcast(qtb, u32)
    if G:
        qtf_scr[...] = qtb.astype(f32)

    zeros = jnp.zeros((128 - DH, TQ), bf16)
    bufs = (sA, sB)
    qbs = (qbA, qbB)
    always = jnp.full((8, 128), i, jnp.int32) >= 0
    always4 = jnp.full((8, TQ), i, jnp.int32) >= 0

    def qk_weights(h, par):
        start = h * DH if isinstance(h, int) else pl.multiple_of(h * DH, DH)
        if G and par is not None:
            qh = qtf_scr[pl.ds(start, DH), :]
            for d in range(DH):
                qbs[par][8 * d:8 * d + 8, :] = jnp.broadcast_to(qh[d:d + 1, :], (8, TQ))
        start2 = h * (DH // 2) if isinstance(h, int) else pl.multiple_of(h * (DH // 2), DH // 2)
        return jnp.concatenate([pltpu.bitcast(qt_scr[pl.ds(start2, DH // 2), :], bf16), zeros], axis=0)

    def qk_chunk(w, c, par, m, mv):
        dst = bufs[par]
        r0, nm = STARTS[c], ROWS[c]
        s = jnp.dot(pltpu.bitcast(kv_scr[r0 // 2:(r0 + nm) // 2, :], bf16), w, preferred_element_type=f32)
        dst[r0:r0 + nm, :] = s
        for r in range(nm // 8):
            sr = s[8 * r:8 * r + 8, :]
            m = sr if m is None else jnp.maximum(m, sr)
        if G:
            j, gq = c % NCT, c // NCT
            k0 = gq * 8 * G
            accs = [None] * G
            for d in range(DH):
                r = (d * (nm // 8)) // DH
                trig = s[8 * r:8 * r + 8, 128 * j:128 * (j + 1)]
                qd = jnp.where(always, qbs[par][8 * d:8 * d + 8, 128 * j:128 * (j + 1)], trig)
                for g in range(G):
                    t = kb_scr[d, k0 + 8 * g:k0 + 8 * g + 8, :] * qd
                    accs[g] = t if accs[g] is None else accs[g] + t
            mv = list(mv)
            for g in range(G):
                dst[k0 + 8 * g:k0 + 8 * g + 8, 128 * j:128 * (j + 1)] = accs[g]
                mv[j] = accs[g] if mv[j] is None else jnp.maximum(mv[j], accs[g])
        return m, mv, s

    def fin_max(m, mv):
        if G:
            m = jnp.maximum(m, jnp.concatenate(mv, axis=1))
        return jnp.max(m, axis=0, keepdims=True)

    def pv_chunk(c, src, m, l, acc, dep):
        mb = jnp.broadcast_to(m, (8, TQ))
        rows_per = CK // NQ
        parts = [None] * NQ
        for q in range(NQ):
            blk = NQ - 1 - q
            trig = dep[q] if dep is not None else None
            mq = mb if trig is None else jnp.where(always4, mb, trig)
            sc = src[c * CK + blk * rows_per:c * CK + (blk + 1) * rows_per, :]
            pq = jnp.exp2(sc.reshape(rows_per // 8, 8, TQ) - mq[None]).reshape(rows_per, TQ)
            for r in reversed(range(rows_per // 8)):
                pr = pq[8 * r:8 * r + 8, :]
                l = pr if l is None else l + pr
            parts[blk] = pq
        p = jnp.concatenate(parts, axis=0)
        o = jnp.dot(pltpu.bitcast(vt_scr[:, c * CK:(c + 1) * CK], bf16), p.astype(bf16), preferred_element_type=f32)
        acc = o if acc is None else acc + o
        return l, acc

    NONE4 = [None] * NCT

    def run_slots(h0, nslots, m_fin, m_part, mv, qk_limit):
        l = acc = None
        w = None
        hist = {}
        for j in range(nslots):
            g = j + LAG
            hq, cq = g // NCK, g % NCK
            if g < qk_limit:
                if cq == 0:
                    w = qk_weights(h0 + hq, hq % 2)
                    m_part, mv = None, NONE4
                elif w is None:
                    w = qk_weights(h0 + hq, None)
                m_part, mv, sval = qk_chunk(w, cq, hq % 2, m_part, mv)
                hist[j] = sval
                if cq == NCK - 1:
                    m_fin[hq] = fin_max(m_part, mv)
                    m_part, mv = None, NONE4
            hp, cp = j // NCK, j % NCK
            if cp == 0:
                l = acc = None
            dep = []
            for q in range(NQ):
                tick = TOFF + (q * TSPAN) // NQ
                if tick < 0:
                    sv = hist.get(j - 2)
                    r = None if sv is None else sv.shape[0] // 8 + tick
                else:
                    sv = hist.get(j - 1)
                    r = tick
                dep.append(None if sv is None else sv[8 * r:8 * r + 8, :])
            l, acc = pv_chunk(cp, bufs[hp % 2], m_fin[hp], l, acc, dep)
            if cp == NCK - 1:
                lt = jnp.sum(l, axis=0, keepdims=True)
                hh = h0 + hp
                start = hh * DH if isinstance(hh, int) else pl.multiple_of(hh * DH, DH)
                ot_scr[pl.ds(start, DH), :] = acc * (1.0 / lt)
        return m_fin, m_part, mv

    m_fin = {}
    m_part, mv = None, NONE4
    w = None
    for g in range(LAG):
        hq, cq = g // NCK, g % NCK
        if cq == 0:
            w = qk_weights(hq, hq % 2); m_part, mv = None, NONE4
        m_part, mv, _ = qk_chunk(w, cq, hq % 2, m_part, mv)
        if cq == NCK - 1:
            m_fin[hq] = fin_max(m_part, mv)
            m_part, mv = None, NONE4

    def pack_mv(mv):
        return [v for v in mv if v is not None]

    def unpack_mv(vals):
        return list(vals) + [None] * (NCT - len(vals))

    def body(it, carry):
        m0, mp, mvv = carry
        h0 = it * HPB
        mf, mp, mvv = run_slots(h0, HPB * NCK, {0: m0}, mp, unpack_mv(mvv), qk_limit=10 ** 9)
        return mf[HPB], mp, pack_mv(mvv)

    nb = H // HPB - 1
    m0, mp, mvv = lax.fori_loop(0, nb, body, (m_fin[0], m_part, pack_mv(mv)))

    @pl.when(i == 0)
    def _():
        for c in copies():
            c.wait()

    run_slots(nb * HPB, HPB * NCK, {0: m0}, mp, unpack_mv(mvv), qk_limit=HPB * NCK)

    o = ot_scr[...].T.astype(bf16)
    a = jnp.dot(o, wo_ref[...], preferred_element_type=f32)

    b = None
    for fc in range(F // FC):
        gch = jnp.dot(xq, wg_ref[:, fc * FC:(fc + 1) * FC], preferred_element_type=f32)
        uch = jnp.dot(xq, wu_ref[:, fc * FC:(fc + 1) * FC], preferred_element_type=f32)
        act = (gch * jax.nn.sigmoid(gch) * uch).astype(bf16)
        bc = jnp.dot(act, wd_ref[fc * FC:(fc + 1) * FC, :], preferred_element_type=f32)
        b = bc if b is None else b + bc

    gw = gw_ref[...].astype(f32).reshape(1, D)
    z = jnp.sum(xq.astype(f32) * gw, axis=-1, keepdims=True)
    g = jax.nn.sigmoid(z)
    o_ref[...] = (g * a + (1.0 - g) * b).astype(o_ref.dtype)


@jax.jit
def pallas_gated_mix__grouped_kv_mqa__swiglu_ffn__prompt_kernel(A_x, A_wq, A_wk, A_wv, A_wo, B_x, B_w_gate, B_w_up, B_w_down, gate_w):
    full = lambda shape: pl.BlockSpec(shape, lambda i: (0,) * len(shape))
    hbm = pl.BlockSpec(memory_space=pl.ANY)
    return pl.pallas_call(
        kernel,
        grid=(S // TQ,),
        in_specs=[
            pl.BlockSpec((None, S, D), lambda i: (0, 0, 0)),
            full((D, D)), full((DH, D)), full((DH, D)), full((D,)),
            hbm, hbm, hbm, hbm,
        ],
        out_specs=pl.BlockSpec((None, TQ, D), lambda i: (0, i, 0)),
        out_shape=jax.ShapeDtypeStruct((1, S, D), bf16),
        scratch_shapes=[
            pltpu.VMEM((128, D), bf16), pltpu.VMEM((S // 2, 128), u32), pltpu.VMEM((DH // 2, S), u32),
            pltpu.VMEM((D, D), bf16), pltpu.VMEM((D // 2, TQ), u32), pltpu.VMEM((D, TQ), f32),
            pltpu.VMEM((S, TQ), f32), pltpu.VMEM((S, TQ), f32),
            pltpu.VMEM((D, D), bf16), pltpu.VMEM((D, F), bf16), pltpu.VMEM((D, F), bf16), pltpu.VMEM((F, D), bf16),
            pltpu.VMEM((DH, max(XV, 8), 128), f32), pltpu.VMEM((D, TQ), f32),
            pltpu.VMEM((8 * DH, TQ), f32), pltpu.VMEM((8 * DH, TQ), f32),
            pltpu.SemaphoreType.DMA((4,)),
        ],
        compiler_params=pltpu.CompilerParams(dimension_semantics=("arbitrary",),
                                             vmem_limit_bytes=100 * 1024 * 1024),
    )(A_x, A_wq, A_wk.T, A_wv.T, gate_w, A_wo, B_w_gate, B_w_up, B_w_down)
```

```python
import math
import jax
import jax.numpy as jnp
from jax import lax
from jax.experimental import pallas as pl
from jax.experimental.pallas import tpu as pltpu

S = 2048; D = 512; H = 32; DH = 16; F = 1792
TQ = 512
CK = 128
NCT = TQ // 128
HPB = 4
NB = H // HPB - 1
FCH = F // NB
XV = 320
XVL = 256
GB = 8
TANH = 1
QSCALE = (DH ** -0.5) * math.log2(math.e)
f32 = jnp.float32; bf16 = jnp.bfloat16; u32 = jnp.uint32
MB = 128
S_MAX = 60.0
V_LO = 2.0 ** -40
V_HI = 2.0 ** 40
FORCE_SLOW = 0
NRB = TQ // MB


def spread(n_extra, n_slots):
    return [((k + 1) * n_slots) // n_extra - 1 for k in range(n_extra)]


def kernel(x_ref, wq_ref, wkt_ref, wvt_ref, gw_ref, wo_hbm, wg_hbm, wu_hbm, wd_hbm, o_ref,
           wkv_scr, kv_scr, vt_scr, wqt_scr, qt_scr, ot_scr, wo_ref, wg_ref, wu_ref, wd_ref,
           kb_scr, qtf_scr, qbA, qbB, pvA, pvB, xq_scr, act_scr, a_scr, b_scr, s_scr, kstat, sems):
    i = pl.program_id(0)

    def chunk_copies(c):
        col = c * FCH if isinstance(c, int) else pl.multiple_of(c * FCH, FCH)
        return [
            pltpu.make_async_copy(wg_hbm.at[:, pl.ds(col, FCH)], wg_ref.at[c], sems.at[3 * c]),
            pltpu.make_async_copy(wu_hbm.at[:, pl.ds(col, FCH)], wu_ref.at[c], sems.at[3 * c + 1]),
            pltpu.make_async_copy(wd_hbm.at[pl.ds(col, FCH), :], wd_ref.at[c], sems.at[3 * c + 2]),
        ]

    def wo_copy():
        return pltpu.make_async_copy(wo_hbm, wo_ref, sems.at[3 * NB])

    @pl.when(i == 0)
    def _():
        for c in range(NB):
            for cp in chunk_copies(c):
                cp.start()
        wo_copy().start()
        wkv_scr[0:DH, :] = wkt_ref[...]
        wkv_scr[DH:2 * DH, :] = wvt_ref[...]
        wkv_scr[2 * DH:, :] = jnp.zeros((128 - 2 * DH, D), bf16)
        kv = lax.dot_general(x_ref[...], wkv_scr[...], (((1,), (1,)), ((), ())), preferred_element_type=f32)
        kvb = kv.astype(bf16)
        kvu = pltpu.bitcast(kvb, u32)
        for c in range(S // CK):
            for g in range(8):
                kv_scr[c * 64 + g * 8:c * 64 + g * 8 + 8, :] = kvu[c * 64 + (7 - g) * 8:c * 64 + (7 - g) * 8 + 8, :]
        kvt = kvb.astype(f32).T
        kt, vt = kvt[0:DH, :], kvt[DH:2 * DH, :]
        vt_scr[...] = pltpu.bitcast(vt.astype(bf16), u32)
        kstat[0] = jnp.max(jnp.sum(kt * kt, axis=0, keepdims=True))
        vcol = jnp.max(jnp.abs(vt), axis=1, keepdims=True)
        v_ok = (vcol == 0.0) | ((vcol >= V_LO) & (vcol <= V_HI))
        kstat[1] = jnp.min(jnp.where(v_ok, 1.0, 0.0))
        wqt_scr[...] = wq_ref[...].astype(f32).T.astype(bf16)
        rows = kvb[:XV, :].astype(f32)
        for d in range(DH):
            kb_scr[d] = jnp.broadcast_to(rows[:, d:d + 1], (XV, 128))

    row0 = pl.multiple_of(i * TQ, TQ)
    xq = x_ref[pl.ds(row0, TQ), :]
    xq_scr[...] = pltpu.bitcast(xq, u32)
    b_scr[...] = jnp.zeros_like(b_scr)
    qt = lax.dot_general(wqt_scr[...], xq, (((1,), (1,)), ((), ())), preferred_element_type=f32)
    qtb = (qt * QSCALE).astype(bf16)
    qt_scr[...] = pltpu.bitcast(qtb, u32)
    qf = qtb.astype(f32)
    qtf_scr[...] = qf
    q2 = qf * qf
    qn = None
    for h in range(H):
        t2 = q2[h * DH:h * DH + 8, :] + q2[h * DH + 8:(h + 1) * DH, :]
        qn = t2 if qn is None else jnp.maximum(qn, t2)
    qmax2 = jnp.max(jnp.sum(qn, axis=0, keepdims=True))
    safe = jnp.logical_and(qmax2 * kstat[0] <= S_MAX * S_MAX, kstat[1] > 0.5)
    if FORCE_SLOW:
        safe = jnp.logical_and(safe, i < 0)

    zeros = jnp.zeros((128 - DH, TQ), bf16)
    qbs = (qbA, qbB)
    pvs = (pvA, pvB)
    always = jnp.full((8, 128), i, jnp.int32) >= 0

    def mo(v, m):
        return v if isinstance(v, int) else pl.multiple_of(v, m)

    def qk_weights(h):
        return jnp.concatenate([pltpu.bitcast(qt_scr[pl.ds(mo(h * 8, 8), 8), :], bf16), zeros], axis=0)

    def fill_qb(h, par):
        qh = qtf_scr[pl.ds(mo(h * DH, DH), DH), :]
        for d in range(DH):
            qbs[par][8 * d:8 * d + 8, :] = jnp.broadcast_to(qh[d:d + 1, :], (8, TQ))

    def vt_tile(t):
        return pltpu.bitcast(vt_scr[:, t * CK:(t + 1) * CK], bf16)

    def qk_tile(w, t, n=CK):
        return jnp.dot(pltpu.bitcast(kv_scr[t * 64:t * 64 + n // 2, :], bf16), w, preferred_element_type=f32)

    def exp_tile(s, l):
        n = s.shape[0] // 16
        p = jnp.exp2(s)
        for r in range(2 * n):
            pr = p[8 * r:8 * r + 8, :]
            l = pr if l is None else l + pr
        pt = jnp.concatenate([p[16 * (n - 1 - g):16 * (n - g), :] for g in range(n)], axis=0).astype(bf16)
        return pt, l

    def finish(h, acc, l):
        lt = jnp.sum(l, axis=0, keepdims=True)
        ot_scr[pl.ds(mo(h * DH, DH), DH), :] = acc * (1.0 / lt)

    def x_rows(rb):
        return pltpu.bitcast(xq_scr[rb * MB // 2:(rb + 1) * MB // 2, :], bf16)

    def ffn_units(it):
        st = {}

        def gate(rb, f):
            def run():
                g = jnp.dot(x_rows(rb), wg_ref[it, :, f * 128:(f + 1) * 128], preferred_element_type=f32)
                if TANH:
                    hg = 0.5 * g
                    st[rb, f] = hg + hg * jnp.tanh(hg)
                else:
                    st[rb, f] = g * jax.nn.sigmoid(g)
                return g
            return run

        def up(rb, f):
            def run():
                u = jnp.dot(x_rows(rb), wu_ref[it, :, f * 128:(f + 1) * 128], preferred_element_type=f32)
                act = (st.pop((rb, f)) * u).astype(bf16)
                k = rb * 2 + f
                act_scr[k * 64:(k + 1) * 64, :] = pltpu.bitcast(act, u32)
                return u
            return run

        def down(rb, f):
            def run():
                k = rb * 2 + f
                act = pltpu.bitcast(act_scr[k * 64:(k + 1) * 64, :], bf16)
                r = jnp.dot(act, wd_ref[it, f * 128:(f + 1) * 128, :], preferred_element_type=f32)
                b_scr[rb * MB:(rb + 1) * MB, :] += r
                return r
            return run

        pieces = [(rb, f) for rb in range(NRB) for f in range(2)]
        units = []
        for n, (rb, f) in enumerate(pieces):
            units += [gate(rb, f), up(rb, f)]
            if n >= 1:
                units.append(down(*pieces[n - 1]))
        units.append(down(*pieces[-1]))
        return units

    def oproj_unit(kt, rb):
        def run():
            o = ot_scr[kt * 128:(kt + 1) * 128, rb * MB:(rb + 1) * MB].T.astype(bf16)
            r = jnp.dot(o, wo_ref[kt * 128:(kt + 1) * 128, :], preferred_element_type=f32)
            if kt == 0:
                a_scr[rb * MB:(rb + 1) * MB, :] = r
            else:
                a_scr[rb * MB:(rb + 1) * MB, :] += r
            return r
        return run

    def heads(h0, lv, units, xvs):
        nh = HPB
        per_head = len(units) // nh
        pend = None
        state = {}
        units = list(units)
        for hr in range(nh):
            par = hr % 2
            xv, xvn = xvs[hr], xvs[hr + 1]
            nvt = xv // CK
            nm = S // CK - nvt
            rows = [CK - (xv - nvt * CK)] + [CK] * (nm - 1)
            fpos = spread(per_head, nm)
            free = [c for c in range(1, nm) if c not in fpos]
            vpos = {free[((t + 1) * len(free)) // (nvt + 1)]: t for t in range(nvt)}
            assert len(vpos) == nvt
            ntick = sum(rows) // 8 + per_head * 16
            nstep = (xvn // (8 * GB)) * NCT * DH
            w = qk_weights(h0 + hr)
            if xvn:
                fill_qb(h0 + hr + 1, 1 - par)
            state[hr] = dict(acc=None, l=jnp.concatenate(lv, axis=1))
            vs = dict(step=0, accs=None, lvn=[None] * NCT, base=0)

            def vpu_steps(val):
                base = vs['base']
                nt = val.shape[0] // 8
                vs['base'] = base + nt
                while vs['step'] < nstep and (vs['step'] * ntick) // nstep < base + nt:
                    step = vs['step']
                    tick = (step * ntick) // nstep - base
                    u, d = step // DH, step % DH
                    j, kb = u % NCT, u // NCT
                    k0 = kb * 8 * GB
                    jj = j % (val.shape[1] // 128)
                    trig = val[8 * tick:8 * tick + 8, 128 * jj:128 * (jj + 1)]
                    qd = jnp.where(always, qbs[1 - par][8 * d:8 * d + 8, 128 * j:128 * (j + 1)], trig)
                    if d == 0:
                        vs['accs'] = [None] * GB
                    accs = vs['accs']
                    for g in range(GB):
                        tt = kb_scr[d, k0 + 8 * g:k0 + 8 * g + 8, :] * qd
                        accs[g] = tt if accs[g] is None else accs[g] + tt
                    if d == DH - 1:
                        ps = [jnp.exp2(a) for a in accs]
                        for pq in ps:
                            vs['lvn'][j] = pq if vs['lvn'][j] is None else vs['lvn'][j] + pq
                        pc = jnp.concatenate(ps, axis=0).astype(bf16)
                        pvs[1 - par][k0 // 2:k0 // 2 + 4 * GB, 128 * j:128 * (j + 1)] = pltpu.bitcast(pc, u32)
                    vs['step'] = step + 1

            for c in range(nm):
                t = nvt + c
                s = qk_tile(w, t, rows[c])
                if c in vpos:
                    tv = vpos[c]
                    pvt = pltpu.bitcast(pvs[par][tv * 64:(tv + 1) * 64, :], bf16)
                    o = jnp.dot(vt_tile(tv), pvt, preferred_element_type=f32)
                    st = state[hr]
                    st['acc'] = o if st['acc'] is None else st['acc'] + o
                if pend is not None:
                    ph, ppt, ptile, plast = pend
                    o = jnp.dot(vt_tile(ptile), ppt, preferred_element_type=f32)
                    st = state[ph]
                    st['acc'] = o if st['acc'] is None else st['acc'] + o
                    if plast:
                        finish(h0 + ph, st['acc'], st['l'])
                pt, state[hr]['l'] = exp_tile(s, state[hr]['l'])
                if rows[c] < CK:
                    nvr = CK - rows[c]
                    pvt = pltpu.bitcast(pvs[par][t * 64:t * 64 + nvr // 2, :], bf16)
                    pt = jnp.concatenate([pvt, pt], axis=0)
                pend = (hr, pt, t, c == nm - 1)
                vpu_steps(s)
                for _ in range(fpos.count(c)):
                    vpu_steps(units.pop(0)())
            assert vs['step'] == nstep
            lv = vs['lvn']
        assert not units
        ph, ppt, ptile, plast = pend
        o = jnp.dot(vt_tile(ptile), ppt, preferred_element_type=f32)
        st = state[ph]
        finish(h0 + ph, st['acc'] + o, st['l'])
        return lv

    def blend(last_kt):
        gw = gw_ref[...].astype(f32).reshape(1, D)
        for rb in range(NRB):
            a = a_scr[rb * MB:(rb + 1) * MB, :]
            if last_kt:
                o = ot_scr[3 * 128:4 * 128, rb * MB:(rb + 1) * MB].T.astype(bf16)
                a = a + jnp.dot(o, wo_ref[3 * 128:4 * 128, :], preferred_element_type=f32)
            z = jnp.sum(x_rows(rb).astype(f32) * gw, axis=-1, keepdims=True)
            g = jax.nn.sigmoid(z)
            o_ref[rb * MB:(rb + 1) * MB, :] = (g * a + (1.0 - g) * b_scr[rb * MB:(rb + 1) * MB, :]).astype(o_ref.dtype)

    @pl.when(safe)
    def _fast():
        w0 = qk_weights(0)
        l0 = None
        for t in range(-(-XV // CK)):
            n = min(CK, XV - t * CK)
            s0 = jnp.dot(pltpu.bitcast(kv_scr[t * 64 + (CK - n) // 2:(t + 1) * 64, :], bf16), w0, preferred_element_type=f32)
            pt, l0 = exp_tile(s0, l0)
            pvA[t * 64:t * 64 + n // 2, :] = pltpu.bitcast(pt, u32)
        lv0 = [l0[:, 128 * j:128 * (j + 1)] for j in range(NCT)]

        def body(it, lv):
            @pl.when(i == 0)
            def _():
                for cp in chunk_copies(it):
                    cp.wait()
            return heads(it * HPB, lv, ffn_units(it), [XV] * (HPB + 1))

        lv = lax.fori_loop(0, NB, body, lv0)

        @pl.when(i == 0)
        def _():
            wo_copy().wait()

        heads(NB * HPB, lv, [oproj_unit(kt, rb) for kt in range(3) for rb in range(NRB)], [XV] + [XVL] * (HPB - 1) + [0])
        blend(True)

    @pl.when(jnp.logical_not(safe))
    def _exact():
        def head(h, carry):
            w = qk_weights(h)

            def pass1(t, m):
                r = pl.multiple_of(t * 64, 64)
                sc = jnp.dot(pltpu.bitcast(kv_scr[pl.ds(r, 64), :], bf16), w, preferred_element_type=f32)
                s_scr[pl.ds(pl.multiple_of(t * CK, CK), CK), :] = sc
                return jnp.maximum(m, jnp.max(sc, axis=0, keepdims=True))

            m = lax.fori_loop(0, S // CK, pass1, jnp.full((1, TQ), -jnp.inf, f32))

            def pass2(t, c):
                l, acc = c
                col = pl.multiple_of(t * CK, CK)
                pt, l = exp_tile(s_scr[pl.ds(col, CK), :] - m, l)
                v = pltpu.bitcast(vt_scr[:, pl.ds(col, CK)], bf16)
                return l, acc + jnp.dot(v, pt, preferred_element_type=f32)

            l, acc = lax.fori_loop(0, S // CK, pass2, (jnp.zeros((8, TQ), f32), jnp.zeros((DH, TQ), f32)))
            finish(h, acc, l)
            return carry

        lax.fori_loop(0, H, head, 0)

        def ffn(it, carry):
            @pl.when(i == 0)
            def _():
                for cp in chunk_copies(it):
                    cp.wait()
            for u in ffn_units(it):
                u()
            return carry

        lax.fori_loop(0, NB, ffn, 0)

        @pl.when(i == 0)
        def _():
            wo_copy().wait()

        a_scr[...] = jnp.dot(ot_scr[...].T.astype(bf16), wo_ref[...], preferred_element_type=f32)
        blend(False)


@jax.jit
def pallas_gated_mix__grouped_kv_mqa__swiglu_ffn__prompt_kernel(A_x, A_wq, A_wk, A_wv, A_wo, B_x, B_w_gate, B_w_up, B_w_down, gate_w):
    full = lambda shape: pl.BlockSpec(shape, lambda i: (0,) * len(shape))
    hbm = pl.BlockSpec(memory_space=pl.ANY)
    return pl.pallas_call(
        kernel,
        grid=(S // TQ,),
        in_specs=[
            pl.BlockSpec((None, S, D), lambda i: (0, 0, 0)),
            full((D, D)), full((DH, D)), full((DH, D)), full((D,)),
            hbm, hbm, hbm, hbm,
        ],
        out_specs=pl.BlockSpec((None, TQ, D), lambda i: (0, i, 0)),
        out_shape=jax.ShapeDtypeStruct((1, S, D), bf16),
        scratch_shapes=[
            pltpu.VMEM((128, D), bf16), pltpu.VMEM((S // 2, 128), u32), pltpu.VMEM((DH // 2, S), u32),
            pltpu.VMEM((D, D), bf16), pltpu.VMEM((D // 2, TQ), u32), pltpu.VMEM((D, TQ), f32),
            pltpu.VMEM((D, D), bf16), pltpu.VMEM((NB, D, FCH), bf16), pltpu.VMEM((NB, D, FCH), bf16),
            pltpu.VMEM((NB, FCH, D), bf16),
            pltpu.VMEM((DH, XV, 128), f32), pltpu.VMEM((D, TQ), f32),
            pltpu.VMEM((8 * DH, TQ), f32), pltpu.VMEM((8 * DH, TQ), f32),
            pltpu.VMEM((XV // 2, TQ), u32), pltpu.VMEM((XV // 2, TQ), u32),
            pltpu.VMEM((TQ // 2, D), u32), pltpu.VMEM((NRB * 2 * 64, 128), u32),
            pltpu.VMEM((TQ, D), f32), pltpu.VMEM((TQ, D), f32),
            pltpu.VMEM((S, TQ), f32), pltpu.SMEM((2,), f32),
            pltpu.SemaphoreType.DMA((3 * NB + 1,)),
        ],
        compiler_params=pltpu.CompilerParams(dimension_semantics=("arbitrary",),
                                             vmem_limit_bytes=100 * 1024 * 1024),
    )(A_x, A_wq, A_wk.T, A_wv.T, gate_w, A_wo, B_w_gate, B_w_up, B_w_down)
```

```python
import math

import jax
import jax.numpy as jnp
from jax import lax
from jax.experimental import pallas as pl
from jax.experimental.pallas import tpu as pltpu

S, D, H, DH, F = 2048, 512, 32, 16, 1792
TQ = 512
CK = 128
MB = 128
NCT = TQ // 128
NRB = TQ // MB
NSTEP = S // TQ
HPB = 4
NB = H // HPB - 1
FCH = F // NB
QSCALE = (DH ** -0.5) * math.log2(math.e)

S_MAX = 60.0
V_LO, V_HI = 2.0 ** -40, 2.0 ** 40

XV = 368
XV_LAST = [336, 336, 336]
XVM = max([XV] + XV_LAST)
LOOP_CFG = dict(gb=8, off=1, tsh=8, fpos=(1, 3, 6, 8, 10, -1), vpos=(5, -2))
LAST_CFG = dict(gb=8, off=2, tsh=0, fpos=(3, 8, -1), vpos=(9, -2))

f32, bf16, u32 = jnp.float32, jnp.bfloat16, jnp.uint32
_NT = (((1,), (1,)), ((), ()))

SEM_WO = NB
SEM_X = NB + 1
SEM_SMALL = SEM_X + NSTEP
SEM_OUT = SEM_SMALL + 4
NSEM = SEM_OUT + NRB


def _kernel(x_hbm, wq_hbm, wkt_hbm, wvt_hbm, gw_hbm, wo_hbm, wg_hbm, wu_hbm, wd_hbm, o_hbm,
            x_ref, wq_ref, gw_ref, wkv_scr, k_scr, vt_scr, wqt_scr, qt_scr, ot_scr,
            wo_ref, wg_ref, wu_ref, wd_ref, kb_scr, qtf_scr, qb_a, qb_b, pv_a, pv_b, xq_scr,
            a_scr, b_scr, s_scr, lv_scr, g_scr, gt_scr, o_scr, stat, sems):
    i = pl.program_id(0)

    def mo(v, m):
        return v if isinstance(v, int) else pl.multiple_of(v, m)

    def chunk_copies(c):
        cps = []
        for f in range(2):
            col = mo(c * FCH + f * 128, 128)
            cps.append(pltpu.make_async_copy(wg_hbm.at[:, pl.ds(col, 128)], wg_ref.at[2 * c + f], sems.at[c]))
            cps.append(pltpu.make_async_copy(wu_hbm.at[:, pl.ds(col, 128)], wu_ref.at[2 * c + f], sems.at[c]))
        row = mo(c * FCH, FCH)
        for j in range(D // 128):
            cps.append(pltpu.make_async_copy(wd_hbm.at[pl.ds(row, FCH), pl.ds(j * 128, 128)],
                                             wd_ref.at[j, pl.ds(row, FCH), :], sems.at[c]))
        return cps

    def wo_copies():
        return [pltpu.make_async_copy(wo_hbm.at[:, pl.ds(j * 128, 128)], wo_ref.at[j], sems.at[SEM_WO])
                for j in range(D // 128)]

    def x_copy(c):
        return pltpu.make_async_copy(x_hbm.at[0, pl.ds(c * TQ, TQ), :], x_ref.at[pl.ds(c * TQ, TQ), :],
                                     sems.at[SEM_X + c])

    def small_copies():
        return [
            pltpu.make_async_copy(wkt_hbm, wkv_scr.at[pl.ds(0, DH), :], sems.at[SEM_SMALL]),
            pltpu.make_async_copy(wvt_hbm, wkv_scr.at[pl.ds(DH, DH), :], sems.at[SEM_SMALL + 1]),
            pltpu.make_async_copy(wq_hbm, wq_ref, sems.at[SEM_SMALL + 2]),
            pltpu.make_async_copy(gw_hbm, gw_ref, sems.at[SEM_SMALL + 3]),
        ]

    def out_copy(step, rb):
        return pltpu.make_async_copy(o_scr.at[pl.ds(rb * MB, MB), :],
                                     o_hbm.at[0, pl.ds(pl.multiple_of(step * TQ + rb * MB, MB), MB), :],
                                     sems.at[SEM_OUT + rb])

    def packed(ref, idx, r0, n):
        return pltpu.bitcast(ref.bitcast(u32)[idx, pl.ds(mo(r0 // 2, 8), n // 2), :], bf16)

    def packed_wide(ref, r0, n):
        return jnp.concatenate([packed(ref, j, r0, n) for j in range(D // 128)], axis=1)

    def kv_block(c):
        kvt = lax.dot_general(wkv_scr[...], x_ref[c * TQ:(c + 1) * TQ, :], _NT,
                              preferred_element_type=f32).astype(bf16)
        vt_scr[:, c * TQ:(c + 1) * TQ] = pltpu.bitcast(kvt[DH:2 * DH, :], u32)
        kvf = kvt.astype(f32)
        kt, vt = kvf[0:DH, :], kvf[DH:2 * DH, :]
        k2 = jnp.sum(kt * kt, axis=0, keepdims=True)
        vabs = jnp.abs(vt)
        krows = jnp.concatenate([kt, jnp.zeros((128 - DH, TQ), f32)], axis=0).T
        ku = pltpu.bitcast(krows.astype(bf16), u32)
        for t in range(TQ // CK):
            for g in range(8):
                r = (c * (TQ // CK) + t) * 64 + g * 8
                k_scr[r:r + 8, :] = ku[t * 64 + (7 - g) * 8:t * 64 + (7 - g) * 8 + 8, :]
        if c == 0:
            for d in range(DH):
                kb_scr[d] = jnp.broadcast_to(krows[:XVM, d:d + 1], (XVM, 128))
        return k2, vabs

    zeros = jnp.zeros((128 - DH, TQ), bf16)
    qbs = (qb_a, qb_b)
    pvs = (pv_a, pv_b)
    always = jnp.full((8, 128), i, jnp.int32) >= 0

    def qk_weights(h):
        return jnp.concatenate([pltpu.bitcast(qt_scr[pl.ds(mo(h * 8, 8), 8), :], bf16), zeros], axis=0)

    def fill_qb(h, par):
        qh = qtf_scr[pl.ds(mo(h * DH, DH), DH), :]
        for d in range(DH):
            qbs[par][8 * d:8 * d + 8, :] = jnp.broadcast_to(qh[d:d + 1, :], (8, TQ))

    def vt_tile(t):
        return pltpu.bitcast(vt_scr[:, t * CK:(t + 1) * CK], bf16)

    def exp_tile(s, l):
        n = s.shape[0] // 16
        p = jnp.exp2(s)
        for r in range(2 * n):
            pr = p[8 * r:8 * r + 8, :]
            l = pr if l is None else l + pr
        pt = jnp.concatenate([p[16 * (n - 1 - g):16 * (n - g), :] for g in range(n)], axis=0).astype(bf16)
        return pt, l

    def q_phase(row0, mid=None, late=None):
        qmax = None
        for j in range(NCT):
            cols = slice(j * 128, (j + 1) * 128)
            xq = x_ref[pl.ds(mo(row0 + j * 128, 128), 128), :]
            xq_scr[j * 64:(j + 1) * 64, :] = pltpu.bitcast(xq, u32)
            qt = lax.dot_general(wqt_scr[...], xq, _NT, preferred_element_type=f32)
            if j == 0 and mid is not None:
                mid()
            gt = jax.nn.sigmoid(qt[D:D + 8, :])
            gt_scr[:, cols] = gt
            g_scr[cols, :] = jnp.concatenate([1.0 - gt] * 16, axis=0).T
            qtb = (qt[0:D, :] * QSCALE).astype(bf16)
            qt_scr[:, cols] = pltpu.bitcast(qtb, u32)
            qf = qtb.astype(f32)
            qtf_scr[:, cols] = qf
            q2 = qf * qf
            qn = None
            for h in range(H):
                t2 = q2[h * DH:h * DH + 8, :] + q2[h * DH + 8:(h + 1) * DH, :]
                qn = t2 if qn is None else jnp.maximum(qn, t2)
            qn = jnp.sum(qn, axis=0, keepdims=True)
            qmax = qn if qmax is None else jnp.maximum(qmax, qn)
        stat[2] = jnp.max(qmax)
        if late is not None:
            late()
        w0 = qk_weights(0)
        l0 = None
        for t in range(-(-XV // CK)):
            n = min(CK, XV - t * CK)
            s0 = jnp.dot(pltpu.bitcast(k_scr[t * 64 + (CK - n) // 2:(t + 1) * 64, :], bf16), w0,
                         preferred_element_type=f32)
            pt, l0 = exp_tile(s0, l0)
            pv_a[t * 64:t * 64 + n // 2, :] = pltpu.bitcast(pt, u32)
        lv_scr[...] = l0

    @pl.when(i == 0)
    def _():
        sm = small_copies()
        sm[2].start()
        x_copy(0).start()
        for cp in (sm[0], sm[1], sm[3]):
            cp.start()
        for c in range(1, NSTEP):
            x_copy(c).start()
        for cp in chunk_copies(0):
            cp.start()
        b_scr[...] = jnp.zeros_like(b_scr)
        sm[2].wait()
        wqt_scr[0:D, :] = wq_ref[...].astype(f32).T.astype(bf16)
        x_copy(0).wait()
        sm[0].wait()
        sm[1].wait()
        sm[3].wait()
        gw = jnp.broadcast_to(gw_ref[...].astype(f32).reshape(1, D), (DH, D))
        wqt_scr[D:D + DH, :] = gw.astype(bf16)
        k2_0, vabs_0 = kv_block(0)

        def rest_kv():
            k2, vabs = k2_0, vabs_0
            for c in range(1, NSTEP):
                x_copy(c).wait()
            for c in range(1, NB):
                for cp in chunk_copies(c):
                    cp.start()
            for cp in wo_copies():
                cp.start()
            for c in range(1, NSTEP):
                a, b = kv_block(c)
                k2 = jnp.maximum(k2, a)
                vabs = jnp.maximum(vabs, b)
            stat[0] = jnp.max(k2)
            vcol = jnp.max(vabs, axis=1, keepdims=True)
            v_ok = (vcol == 0.0) | ((vcol >= V_LO) & (vcol <= V_HI))
            stat[1] = jnp.min(jnp.where(v_ok, 1.0, 0.0))

        q_phase(0, None, rest_kv)

    safe = jnp.logical_and(stat[2] * stat[0] <= S_MAX * S_MAX, stat[1] > 0.5)

    def finish(h, acc, l):
        lt = jnp.sum(l, axis=0, keepdims=True)
        ot_scr[pl.ds(mo(h * DH, DH), DH), :] = acc * (gt_scr[0:1, :] / lt)

    def x_rows(rb):
        return pltpu.bitcast(xq_scr[rb * MB // 2:(rb + 1) * MB // 2, :], bf16)

    def ffn_units(c):
        st = {}

        def gate(rb, f):
            def unit():
                g = jnp.dot(x_rows(rb), packed(wg_ref, 2 * c + f, 0, D), preferred_element_type=f32)
                hg = 0.5 * g
                st[rb, f] = hg + hg * jnp.tanh(hg)
                return g
            return unit

        def up(rb, f):
            def unit():
                u = jnp.dot(x_rows(rb), packed(wu_ref, 2 * c + f, 0, D), preferred_element_type=f32)
                st['act', rb, f] = (st.pop((rb, f)) * u).astype(bf16)
                return u
            return unit

        def down(rb, f):
            def unit():
                act = st.pop(('act', rb, f))
                r = jnp.dot(act, packed_wide(wd_ref, c * FCH + f * 128, 128), preferred_element_type=f32)
                b_scr[rb * MB:(rb + 1) * MB, :] += r
                return r
            return unit

        pieces = [(rb, f) for rb in range(NRB) for f in range(2)]
        units = []
        for n, (rb, f) in enumerate(pieces):
            units += [gate(rb, f), up(rb, f)]
            if n >= 1:
                units.append(down(*pieces[n - 1]))
        units.append(down(*pieces[-1]))
        return units

    def oproj_units():
        def make(kt, rb):
            def unit():
                rows = slice(rb * MB, (rb + 1) * MB)
                o = ot_scr[kt * 128:(kt + 1) * 128, rows].T.astype(bf16)
                r = jnp.dot(o, packed_wide(wo_ref, kt * 128, 128), preferred_element_type=f32)
                if kt == 1:
                    a_scr[rows, :] = r
                elif kt == 2:
                    a_scr[rows, :] += r
                else:
                    gm = jnp.concatenate([g_scr[rows, :]] * (D // 128), axis=1)
                    a_scr[rows, :] += r + gm * b_scr[rows, :]
                    b_scr[rows, :] = jnp.zeros((MB, D), f32)
                return r
            return unit
        return [make(kt, rb) for kt in (1, 2, 0) for rb in range(NRB)]

    def heads(h0, lv, units, xvs, gb, off, tsh, fpos, vpos):
        per_head = len(units) // HPB
        assert per_head == len(fpos)
        units = list(units)
        pend = None
        state = {}
        ticks = []
        for hr in range(HPB):
            par = hr % 2
            xv, xvn = xvs[hr], xvs[hr + 1]
            nvt = xv // CK
            nm = S // CK - nvt
            rows = [CK - (xv - nvt * CK)] + [CK] * (nm - 1)
            fslots = [v % nm for v in fpos]
            vslots = {vpos[t] % nm: t for t in range(nvt)}
            ntick = sum(rows) // 8 + per_head * 16
            ng = xvn // 8
            nblk = -(-ng // gb)
            sched, cost = [], 0
            for bi in range(nblk):
                g0, g1 = 2 * ((bi * ng // 2) // nblk), 2 * (((bi + 1) * ng // 2) // nblk)
                for j in range(NCT):
                    for d in range(DH):
                        sched.append((g0, g1 - g0, j, d, cost))
                        cost += 2 * (g1 - g0) + 1 + (2 * (g1 - g0) if d == DH - 1 else 0)
            w = qk_weights(h0 + hr)
            if xvn:
                fill_qb(h0 + hr + 1, 1 - par)
            state[hr] = dict(acc=None, l=jnp.concatenate(lv, axis=1))
            vs = dict(step=0, accs=None, lvn=[None] * NCT)
            tick0 = len(ticks) - tsh

            def vpu_steps(val):
                for r in range(val.shape[0] // 8):
                    ticks.append((val, r))
                while vs['step'] < len(sched) and tick0 + (sched[vs['step']][4] * ntick) // cost < len(ticks):
                    g0, n, j, d, c0 = sched[vs['step']]
                    tick = tick0 + (c0 * ntick) // cost
                    k0 = g0 * 8
                    qd = qbs[1 - par][8 * d:8 * d + 8, 128 * j:128 * (j + 1)]
                    if tick >= 0:
                        tv, tr = ticks[tick]
                        jj = j % (tv.shape[1] // 128)
                        qd = jnp.where(always, qd, tv[8 * tr:8 * tr + 8, 128 * jj:128 * (jj + 1)])
                    if d == 0:
                        vs['accs'] = [None] * n
                    accs = vs['accs']
                    for g in range(n):
                        tt = kb_scr[d, k0 + 8 * g:k0 + 8 * g + 8, :] * qd
                        accs[g] = tt if accs[g] is None else accs[g] + tt
                    if d == DH - 1:
                        ps = [jnp.exp2(a) for a in accs]
                        for pq in ps:
                            vs['lvn'][j] = pq if vs['lvn'][j] is None else vs['lvn'][j] + pq
                        pc = jnp.concatenate(ps, axis=0).astype(bf16)
                        pvs[1 - par][k0 // 2:k0 // 2 + 4 * n, 128 * j:128 * (j + 1)] = pltpu.bitcast(pc, u32)
                    vs['step'] += 1

            def add_pv(st, tile_idx, p_tile):
                o = jnp.dot(vt_tile(tile_idx), p_tile, preferred_element_type=f32)
                st['acc'] = o if st['acc'] is None else st['acc'] + o

            stream = [(nvt + c, g) for c in range(nm) for g in range(rows[c] // 16)]
            bounds = [0] + [min(sum(rows[:c + 1]) // 16 + off, len(stream)) for c in range(nm)]
            parts = {}
            for c in range(nm):
                grp = stream[bounds[c]:bounds[c + 1]]
                runs = []
                for (t, g) in grp:
                    r = t * 64 + g * 8
                    if runs and runs[-1][1] == r:
                        runs[-1][1] = r + 8
                    else:
                        runs.append([r, r + 8])
                lhs = [k_scr[r0:r1, :] for r0, r1 in runs]
                lhs = lhs[0] if len(lhs) == 1 else jnp.concatenate(lhs, axis=0)
                s = jnp.dot(pltpu.bitcast(lhs, bf16), w, preferred_element_type=f32)
                if c in vslots:
                    tv = vslots[c]
                    add_pv(state[hr], tv, pltpu.bitcast(pvs[par][tv * 64:(tv + 1) * 64, :], bf16))
                if pend is not None:
                    ph, ppt, ptile, plast = pend
                    add_pv(state[ph], ptile, ppt)
                    if plast:
                        finish(h0 + ph, state[ph]['acc'], state[ph]['l'])
                p = jnp.exp2(s)
                for n, (t, g) in enumerate(grp):
                    for r in (2 * n, 2 * n + 1):
                        state[hr]['l'] = state[hr]['l'] + p[8 * r:8 * r + 8, :]
                    parts.setdefault(t, []).append(p[16 * n:16 * n + 16, :])
                t = nvt + c
                tile = jnp.concatenate(parts.pop(t)[::-1], axis=0).astype(bf16)
                if rows[c] < CK:
                    nvr = CK - rows[c]
                    tile = jnp.concatenate([pltpu.bitcast(pvs[par][t * 64:t * 64 + nvr // 2, :], bf16), tile], axis=0)
                pend = (hr, tile, t, c == nm - 1)
                vpu_steps(s)
                for _ in range(fslots.count(c)):
                    vpu_steps(units.pop(0)())
            assert vs['step'] == len(sched)
            lv = vs['lvn']
        assert not units
        ph, ppt, ptile, _ = pend
        o = jnp.dot(vt_tile(ptile), ppt, preferred_element_type=f32)
        finish(h0 + ph, state[ph]['acc'] + o, state[ph]['l'])
        return lv

    def wait_first(copies):
        @pl.when(i == 0)
        def _():
            for cp in copies:
                cp.wait()

    @pl.when(safe)
    def _fast():
        lv0 = [lv_scr[:, 128 * j:128 * (j + 1)] for j in range(NCT)]

        def body(it, lv):
            wait_first(chunk_copies(it))
            return heads(it * HPB, lv, ffn_units(it), [XV] * (HPB + 1), **LOOP_CFG)

        lv = lax.fori_loop(0, NB, body, lv0)
        wait_first(wo_copies())
        heads(NB * HPB, lv, oproj_units(), [XV] + XV_LAST + [0], **LAST_CFG)

    @pl.when(jnp.logical_not(safe))
    def _exact():
        def head(h, carry):
            w = qk_weights(h)
            m = None
            for t in range(S // CK):
                sc = jnp.dot(pltpu.bitcast(k_scr[t * 64:(t + 1) * 64, :], bf16), w, preferred_element_type=f32)
                s_scr[t * CK:(t + 1) * CK, :] = sc
                for r in range(CK // 8):
                    sr = sc[8 * r:8 * r + 8, :]
                    m = sr if m is None else jnp.maximum(m, sr)
            m = jnp.max(m, axis=0, keepdims=True)
            l = acc = None
            for t in range(S // CK):
                pt, l = exp_tile(s_scr[t * CK:(t + 1) * CK, :] - m, l)
                o = jnp.dot(vt_tile(t), pt, preferred_element_type=f32)
                acc = o if acc is None else acc + o
            finish(h, acc, l)
            return carry

        lax.fori_loop(0, H, head, 0)

        def ffn(it, carry):
            wait_first(chunk_copies(it))
            for unit in ffn_units(it):
                unit()
            return carry

        lax.fori_loop(0, NB, ffn, 0)
        wait_first(wo_copies())
        for unit in oproj_units():
            unit()

    def tail():
        for rb in range(NRB):
            rows = slice(rb * MB, (rb + 1) * MB)
            o = ot_scr[3 * 128:4 * 128, rows].T.astype(bf16)
            r = jnp.dot(o, packed_wide(wo_ref, 3 * 128, 128), preferred_element_type=f32)
            o_scr[rows, :] = (a_scr[rows, :] + r).astype(bf16)
            out_copy(i, rb).start()

    @pl.when(i > 0)
    def _():
        for rb in range(NRB):
            out_copy(i - 1, rb).wait()

    @pl.when(i < NSTEP - 1)
    def _():
        q_phase((i + 1) * TQ, tail)

    @pl.when(i == NSTEP - 1)
    def _():
        tail()
        for rb in range(NRB):
            out_copy(i, rb).wait()


@jax.jit
def pallas_gated_mix__grouped_kv_mqa__swiglu_ffn__prompt_kernel(
    A_x, A_wq, A_wk, A_wv, A_wo, B_x, B_w_gate, B_w_up, B_w_down, gate_w
):
    hbm = pl.BlockSpec(memory_space=pl.ANY)
    vmem = pltpu.VMEM
    return pl.pallas_call(
        _kernel,
        grid=(NSTEP,),
        in_specs=[hbm] * 9,
        out_specs=hbm,
        out_shape=jax.ShapeDtypeStruct((1, S, D), bf16),
        scratch_shapes=[
            vmem((S, D), bf16),
            vmem((D, D), bf16),
            vmem((D,), bf16),
            vmem((2 * DH, D), bf16),
            vmem((S // 2, 128), u32),
            vmem((DH // 2, S), u32),
            vmem((D + DH, D), bf16),
            vmem((D // 2, TQ), u32),
            vmem((D, TQ), f32),
            vmem((D // 128, D, 128), bf16),
            vmem((F // 128, D, 128), bf16),
            vmem((F // 128, D, 128), bf16),
            vmem((D // 128, F, 128), bf16),
            vmem((DH, XVM, 128), f32),
            vmem((D, TQ), f32),
            vmem((8 * DH, TQ), f32),
            vmem((8 * DH, TQ), f32),
            vmem((XVM // 2, TQ), u32),
            vmem((XVM // 2, TQ), u32),
            vmem((TQ // 2, D), u32),
            vmem((TQ, D), f32),
            vmem((TQ, D), f32),
            vmem((S, TQ), f32),
            vmem((8, TQ), f32),
            vmem((TQ, 128), f32),
            vmem((8, TQ), f32),
            vmem((TQ, D), bf16),
            pltpu.SMEM((3,), f32),
            pltpu.SemaphoreType.DMA((NSEM,)),
        ],
        compiler_params=pltpu.CompilerParams(
            dimension_semantics=("arbitrary",), vmem_limit_bytes=100 * 1024 * 1024),
    )(A_x, A_wq, A_wk.T, A_wv.T, gate_w, A_wo, B_w_gate, B_w_up, B_w_down)
```

```python
import math

import jax
import jax.numpy as jnp
from jax import lax
from jax.experimental import pallas as pl
from jax.experimental.pallas import tpu as pltpu

S, D, H, DH, F = 2048, 512, 32, 16, 1792
TQ = 512
CK = 128
MB = 128
NCT = TQ // 128
NRB = TQ // MB
NSTEP = S // TQ
HPB = 4
NB = H // HPB - 1
FCH = F // NB
QSCALE = (DH ** -0.5) * math.log2(math.e)

S_MAX = 60.0
V_LO, V_HI = 2.0 ** -40, 2.0 ** 40

XV = 368
XV_LAST = [336, 336, 336]
XVM = max([XV] + XV_LAST)
LOOP_CFG = dict(gb=8, off=1, tsh=8, fpos=(1, 3, 6, 8, 11, -1), vpos=(10, -2))
LAST_CFG = dict(gb=8, off=2, tsh=0, fpos=(3, 8, -1), vpos=(9, -2))

f32, bf16, u32 = jnp.float32, jnp.bfloat16, jnp.uint32
_NT = (((1,), (1,)), ((), ()))

SEM_WO = NB
SEM_X = NB + 1
SEM_SMALL = SEM_X + NSTEP
SEM_OUT = SEM_SMALL + 4
NSEM = SEM_OUT + NRB


def _kernel(x_hbm, wq_hbm, wkt_hbm, wvt_hbm, gw_hbm, wo_hbm, wg_hbm, wu_hbm, wd_hbm, o_hbm,
            x_ref, wq_ref, gw_ref, wkv_scr, k_scr, vt_scr, wqt_scr, qt_scr, ot_scr,
            wo_ref, wg_ref, wu_ref, wd_ref, kb_scr, qtf_scr, qb_a, qb_b, pv_a, pv_b, xq_scr,
            a_scr, b_scr, s_scr, lv_scr, g_scr, gt_scr, o_scr, stat, sems):
    i = pl.program_id(0)

    def mo(v, m):
        return v if isinstance(v, int) else pl.multiple_of(v, m)

    def chunk_copies(c):
        cps = []
        for f in range(2):
            col = mo(c * FCH + f * 128, 128)
            cps.append(pltpu.make_async_copy(wg_hbm.at[:, pl.ds(col, 128)], wg_ref.at[2 * c + f], sems.at[c]))
            cps.append(pltpu.make_async_copy(wu_hbm.at[:, pl.ds(col, 128)], wu_ref.at[2 * c + f], sems.at[c]))
        row = mo(c * FCH, FCH)
        for j in range(D // 128):
            cps.append(pltpu.make_async_copy(wd_hbm.at[pl.ds(row, FCH), pl.ds(j * 128, 128)],
                                             wd_ref.at[j, pl.ds(row, FCH), :], sems.at[c]))
        return cps

    def wo_copies():
        return [pltpu.make_async_copy(wo_hbm.at[:, pl.ds(j * 128, 128)], wo_ref.at[j], sems.at[SEM_WO])
                for j in range(D // 128)]

    def x_copy(c):
        return pltpu.make_async_copy(x_hbm.at[0, pl.ds(c * TQ, TQ), :], x_ref.at[pl.ds(c * TQ, TQ), :],
                                     sems.at[SEM_X + c])

    def small_copies():
        return [
            pltpu.make_async_copy(wkt_hbm, wkv_scr.at[pl.ds(0, DH), :], sems.at[SEM_SMALL]),
            pltpu.make_async_copy(wvt_hbm, wkv_scr.at[pl.ds(DH, DH), :], sems.at[SEM_SMALL + 1]),
            pltpu.make_async_copy(wq_hbm, wq_ref, sems.at[SEM_SMALL + 2]),
            pltpu.make_async_copy(gw_hbm, gw_ref, sems.at[SEM_SMALL + 3]),
        ]

    def out_copy(step, rb):
        return pltpu.make_async_copy(o_scr.at[pl.ds(rb * MB, MB), :],
                                     o_hbm.at[0, pl.ds(pl.multiple_of(step * TQ + rb * MB, MB), MB), :],
                                     sems.at[SEM_OUT + rb])

    def packed(ref, idx, r0, n):
        return pltpu.bitcast(ref.bitcast(u32)[idx, pl.ds(mo(r0 // 2, 8), n // 2), :], bf16)

    def packed_wide(ref, r0, n):
        return jnp.concatenate([packed(ref, j, r0, n) for j in range(D // 128)], axis=1)

    def kv_block(c):
        kvt = lax.dot_general(wkv_scr[...], x_ref[c * TQ:(c + 1) * TQ, :], _NT,
                              preferred_element_type=f32).astype(bf16)
        vt_scr[:, c * TQ:(c + 1) * TQ] = pltpu.bitcast(kvt[DH:2 * DH, :], u32)
        kvf = kvt.astype(f32)
        kt, vt = kvf[0:DH, :], kvf[DH:2 * DH, :]
        k2 = jnp.sum(kt * kt, axis=0, keepdims=True)
        vabs = jnp.abs(vt)
        krows = jnp.concatenate([kt, jnp.zeros((128 - DH, TQ), f32)], axis=0).T
        ku = pltpu.bitcast(krows.astype(bf16), u32)
        for t in range(TQ // CK):
            for g in range(8):
                r = (c * (TQ // CK) + t) * 64 + g * 8
                k_scr[r:r + 8, :] = ku[t * 64 + (7 - g) * 8:t * 64 + (7 - g) * 8 + 8, :]
        if c == 0:
            for d in range(DH):
                kb_scr[d] = jnp.broadcast_to(krows[:XVM, d:d + 1], (XVM, 128))
        return k2, vabs

    zeros = jnp.zeros((128 - DH, TQ), bf16)
    qbs = (qb_a, qb_b)
    pvs = (pv_a, pv_b)
    always = jnp.full((8, 128), i, jnp.int32) >= 0

    def qk_weights(h):
        return jnp.concatenate([pltpu.bitcast(qt_scr[pl.ds(mo(h * 8, 8), 8), :], bf16), zeros], axis=0)

    def fill_qb(h, par):
        qh = qtf_scr[pl.ds(mo(h * DH, DH), DH), :]
        for d in range(DH):
            qbs[par][8 * d:8 * d + 8, :] = jnp.broadcast_to(qh[d:d + 1, :], (8, TQ))

    def vt_tile(t):
        return pltpu.bitcast(vt_scr[:, t * CK:(t + 1) * CK], bf16)

    def exp_tile(s, l):
        n = s.shape[0] // 16
        p = jnp.exp2(s)
        for r in range(2 * n):
            pr = p[8 * r:8 * r + 8, :]
            l = pr if l is None else l + pr
        pt = jnp.concatenate([p[16 * (n - 1 - g):16 * (n - g), :] for g in range(n)], axis=0).astype(bf16)
        return pt, l

    def q_phase(row0, mid=None, late=None):
        qmax = None
        for j in range(NCT):
            cols = slice(j * 128, (j + 1) * 128)
            xq = x_ref[pl.ds(mo(row0 + j * 128, 128), 128), :]
            xq_scr[j * 64:(j + 1) * 64, :] = pltpu.bitcast(xq, u32)
            qt = lax.dot_general(wqt_scr[...], xq, _NT, preferred_element_type=f32)
            if j == 0 and mid is not None:
                mid()
            gt = jax.nn.sigmoid(qt[D:D + 8, :])
            gt_scr[:, cols] = gt
            g_scr[cols, :] = jnp.concatenate([1.0 - gt] * 16, axis=0).T
            qtb = (qt[0:D, :] * QSCALE).astype(bf16)
            qt_scr[:, cols] = pltpu.bitcast(qtb, u32)
            qf = qtb.astype(f32)
            qtf_scr[:, cols] = qf
            q2 = qf * qf
            qn = None
            for h in range(H):
                t2 = q2[h * DH:h * DH + 8, :] + q2[h * DH + 8:(h + 1) * DH, :]
                qn = t2 if qn is None else jnp.maximum(qn, t2)
            qn = jnp.sum(qn, axis=0, keepdims=True)
            qmax = qn if qmax is None else jnp.maximum(qmax, qn)
        stat[2] = jnp.max(qmax)
        if late is not None:
            late()
        w0 = qk_weights(0)
        l0 = None
        for t in range(-(-XV // CK)):
            n = min(CK, XV - t * CK)
            s0 = jnp.dot(pltpu.bitcast(k_scr[t * 64 + (CK - n) // 2:(t + 1) * 64, :], bf16), w0,
                         preferred_element_type=f32)
            pt, l0 = exp_tile(s0, l0)
            pv_a[t * 64:t * 64 + n // 2, :] = pltpu.bitcast(pt, u32)
        lv_scr[...] = l0

    @pl.when(i == 0)
    def _():
        sm = small_copies()
        sm[2].start()
        x_copy(0).start()
        for cp in (sm[0], sm[1], sm[3]):
            cp.start()
        for c in range(1, NSTEP):
            x_copy(c).start()
        for cp in chunk_copies(0):
            cp.start()
        b_scr[...] = jnp.zeros_like(b_scr)
        sm[2].wait()
        wqt_scr[0:D, :] = wq_ref[...].astype(f32).T.astype(bf16)
        x_copy(0).wait()
        sm[0].wait()
        sm[1].wait()
        sm[3].wait()
        gw = jnp.broadcast_to(gw_ref[...].astype(f32).reshape(1, D), (DH, D))
        wqt_scr[D:D + DH, :] = gw.astype(bf16)
        k2_0, vabs_0 = kv_block(0)

        def rest_kv():
            k2, vabs = k2_0, vabs_0
            for c in range(1, NSTEP):
                x_copy(c).wait()
            for c in range(1, NB):
                for cp in chunk_copies(c):
                    cp.start()
            for cp in wo_copies():
                cp.start()
            for c in range(1, NSTEP):
                a, b = kv_block(c)
                k2 = jnp.maximum(k2, a)
                vabs = jnp.maximum(vabs, b)
            stat[0] = jnp.max(k2)
            vcol = jnp.max(vabs, axis=1, keepdims=True)
            v_ok = (vcol == 0.0) | ((vcol >= V_LO) & (vcol <= V_HI))
            stat[1] = jnp.min(jnp.where(v_ok, 1.0, 0.0))

        q_phase(0, None, rest_kv)

    safe = jnp.logical_and(stat[2] * stat[0] <= S_MAX * S_MAX, stat[1] > 0.5)

    def finish(h, acc, l):
        lt = jnp.sum(l, axis=0, keepdims=True)
        ot_scr[pl.ds(mo(h * DH, DH), DH), :] = acc * (gt_scr[0:1, :] / lt)

    def x_rows(rb):
        return pltpu.bitcast(xq_scr[rb * MB // 2:(rb + 1) * MB // 2, :], bf16)

    def ffn_units(c):
        st = {}

        def gate(rb, f):
            def unit():
                g = jnp.dot(x_rows(rb), packed(wg_ref, 2 * c + f, 0, D), preferred_element_type=f32)
                hg = 0.5 * g
                st[rb, f] = hg + hg * jnp.tanh(hg)
                return g
            return unit

        def up(rb, f):
            def unit():
                u = jnp.dot(x_rows(rb), packed(wu_ref, 2 * c + f, 0, D), preferred_element_type=f32)
                st['act', rb, f] = (st.pop((rb, f)) * u).astype(bf16)
                return u
            return unit

        def down(rb, f):
            def unit():
                act = st.pop(('act', rb, f))
                r = jnp.dot(act, packed_wide(wd_ref, c * FCH + f * 128, 128), preferred_element_type=f32)
                b_scr[rb * MB:(rb + 1) * MB, :] += r
                return r
            return unit

        pieces = [(rb, f) for rb in range(NRB) for f in range(2)]
        units = []
        for n, (rb, f) in enumerate(pieces):
            units += [gate(rb, f), up(rb, f)]
            if n >= 1:
                units.append(down(*pieces[n - 1]))
        units.append(down(*pieces[-1]))
        return units

    def oproj_units():
        def make(kt, rb):
            def unit():
                rows = slice(rb * MB, (rb + 1) * MB)
                o = ot_scr[kt * 128:(kt + 1) * 128, rows].T.astype(bf16)
                r = jnp.dot(o, packed_wide(wo_ref, kt * 128, 128), preferred_element_type=f32)
                if kt == 1:
                    a_scr[rows, :] = r
                elif kt == 2:
                    a_scr[rows, :] += r
                else:
                    gm = jnp.concatenate([g_scr[rows, :]] * (D // 128), axis=1)
                    a_scr[rows, :] += r + gm * b_scr[rows, :]
                    b_scr[rows, :] = jnp.zeros((MB, D), f32)
                return r
            return unit
        return [make(kt, rb) for kt in (1, 2, 0) for rb in range(NRB)]

    def heads(h0, lv, units, xvs, gb, off, tsh, fpos, vpos):
        per_head = len(units) // HPB
        assert per_head == len(fpos)
        units = list(units)
        pend = None
        state = {}
        ticks = []
        for hr in range(HPB):
            par = hr % 2
            xv, xvn = xvs[hr], xvs[hr + 1]
            nvt = xv // CK
            nm = S // CK - nvt
            rows = [CK - (xv - nvt * CK)] + [CK] * (nm - 1)
            fslots = [v % nm for v in fpos]
            vslots = {vpos[t] % nm: t for t in range(nvt)}
            ntick = sum(rows) // 8 + per_head * 16
            ng = xvn // 8
            nblk = -(-ng // gb)
            sched, cost = [], 0
            for bi in range(nblk):
                g0, g1 = 2 * ((bi * ng // 2) // nblk), 2 * (((bi + 1) * ng // 2) // nblk)
                for j in range(NCT):
                    for d in range(DH):
                        sched.append((g0, g1 - g0, j, d, cost))
                        cost += 2 * (g1 - g0) + 1 + (2 * (g1 - g0) if d == DH - 1 else 0)
            w = qk_weights(h0 + hr)
            if xvn:
                fill_qb(h0 + hr + 1, 1 - par)
            state[hr] = dict(acc=None, l=jnp.concatenate(lv, axis=1))
            vs = dict(step=0, acc=None, lvn=[None] * NCT)
            tick0 = len(ticks) - tsh

            def vpu_steps(val):
                for r in range(val.shape[0] // 8):
                    ticks.append((val, r))
                while vs['step'] < len(sched) and tick0 + (sched[vs['step']][4] * ntick) // cost < len(ticks):
                    g0, n, j, d, c0 = sched[vs['step']]
                    tick = tick0 + (c0 * ntick) // cost
                    k0 = g0 * 8
                    qd = qbs[1 - par][8 * d:8 * d + 8, 128 * j:128 * (j + 1)]
                    if tick >= 0:
                        tv, tr = ticks[tick]
                        jj = j % (tv.shape[1] // 128)
                        qd = jnp.where(always, qd, tv[8 * tr:8 * tr + 8, 128 * jj:128 * (jj + 1)])
                    tt = kb_scr[d, k0:k0 + 8 * n, :].reshape(n, 8, 128) * qd[None]
                    vs['acc'] = tt if d == 0 else vs['acc'] + tt
                    if d == DH - 1:
                        ps = jnp.exp2(vs['acc'])
                        for g in range(n):
                            vs['lvn'][j] = ps[g] if vs['lvn'][j] is None else vs['lvn'][j] + ps[g]
                        pc = ps.reshape(8 * n, 128).astype(bf16)
                        pvs[1 - par][k0 // 2:k0 // 2 + 4 * n, 128 * j:128 * (j + 1)] = pltpu.bitcast(pc, u32)
                    vs['step'] += 1

            def add_pv(st, tile_idx, p_tile):
                o = jnp.dot(vt_tile(tile_idx), p_tile, preferred_element_type=f32)
                st['acc'] = o if st['acc'] is None else st['acc'] + o

            stream = [(nvt + c, g) for c in range(nm) for g in range(rows[c] // 16)]
            bounds = [0] + [min(sum(rows[:c + 1]) // 16 + off, len(stream)) for c in range(nm)]
            parts = {}
            for c in range(nm):
                grp = stream[bounds[c]:bounds[c + 1]]
                runs = []
                for (t, g) in grp:
                    r = t * 64 + g * 8
                    if runs and runs[-1][1] == r:
                        runs[-1][1] = r + 8
                    else:
                        runs.append([r, r + 8])
                lhs = [k_scr[r0:r1, :] for r0, r1 in runs]
                lhs = lhs[0] if len(lhs) == 1 else jnp.concatenate(lhs, axis=0)
                s = jnp.dot(pltpu.bitcast(lhs, bf16), w, preferred_element_type=f32)
                if c in vslots:
                    tv = vslots[c]
                    add_pv(state[hr], tv, pltpu.bitcast(pvs[par][tv * 64:(tv + 1) * 64, :], bf16))
                if pend is not None:
                    ph, ppt, ptile, plast = pend
                    add_pv(state[ph], ptile, ppt)
                    if plast:
                        finish(h0 + ph, state[ph]['acc'], state[ph]['l'])
                p = jnp.exp2(s)
                for n, (t, g) in enumerate(grp):
                    for r in (2 * n, 2 * n + 1):
                        state[hr]['l'] = state[hr]['l'] + p[8 * r:8 * r + 8, :]
                    parts.setdefault(t, []).append(p[16 * n:16 * n + 16, :])
                t = nvt + c
                tile = jnp.concatenate(parts.pop(t)[::-1], axis=0).astype(bf16)
                if rows[c] < CK:
                    nvr = CK - rows[c]
                    tile = jnp.concatenate([pltpu.bitcast(pvs[par][t * 64:t * 64 + nvr // 2, :], bf16), tile], axis=0)
                pend = (hr, tile, t, c == nm - 1)
                vpu_steps(s)
                for _ in range(fslots.count(c)):
                    vpu_steps(units.pop(0)())
            assert vs['step'] == len(sched)
            lv = vs['lvn']
        assert not units
        ph, ppt, ptile, _ = pend
        o = jnp.dot(vt_tile(ptile), ppt, preferred_element_type=f32)
        finish(h0 + ph, state[ph]['acc'] + o, state[ph]['l'])
        return lv

    def wait_first(copies):
        @pl.when(i == 0)
        def _():
            for cp in copies:
                cp.wait()

    @pl.when(safe)
    def _fast():
        lv0 = [lv_scr[:, 128 * j:128 * (j + 1)] for j in range(NCT)]

        def body(it, lv):
            wait_first(chunk_copies(it))
            return heads(it * HPB, lv, ffn_units(it), [XV] * (HPB + 1), **LOOP_CFG)

        lv = lax.fori_loop(0, NB, body, lv0)
        wait_first(wo_copies())
        heads(NB * HPB, lv, oproj_units(), [XV] + XV_LAST + [0], **LAST_CFG)

    @pl.when(jnp.logical_not(safe))
    def _exact():
        def head(h, carry):
            w = qk_weights(h)
            m = None
            for t in range(S // CK):
                sc = jnp.dot(pltpu.bitcast(k_scr[t * 64:(t + 1) * 64, :], bf16), w, preferred_element_type=f32)
                s_scr[t * CK:(t + 1) * CK, :] = sc
                for r in range(CK // 8):
                    sr = sc[8 * r:8 * r + 8, :]
                    m = sr if m is None else jnp.maximum(m, sr)
            m = jnp.max(m, axis=0, keepdims=True)
            l = acc = None
            for t in range(S // CK):
                pt, l = exp_tile(s_scr[t * CK:(t + 1) * CK, :] - m, l)
                o = jnp.dot(vt_tile(t), pt, preferred_element_type=f32)
                acc = o if acc is None else acc + o
            finish(h, acc, l)
            return carry

        lax.fori_loop(0, H, head, 0)

        def ffn(it, carry):
            wait_first(chunk_copies(it))
            for unit in ffn_units(it):
                unit()
            return carry

        lax.fori_loop(0, NB, ffn, 0)
        wait_first(wo_copies())
        for unit in oproj_units():
            unit()

    def tail():
        for rb in range(NRB):
            rows = slice(rb * MB, (rb + 1) * MB)
            o = ot_scr[3 * 128:4 * 128, rows].T.astype(bf16)
            r = jnp.dot(o, packed_wide(wo_ref, 3 * 128, 128), preferred_element_type=f32)
            o_scr[rows, :] = (a_scr[rows, :] + r).astype(bf16)
            out_copy(i, rb).start()

    @pl.when(i > 0)
    def _():
        for rb in range(NRB):
            out_copy(i - 1, rb).wait()

    @pl.when(i < NSTEP - 1)
    def _():
        q_phase((i + 1) * TQ, tail)

    @pl.when(i == NSTEP - 1)
    def _():
        tail()
        for rb in range(NRB):
            out_copy(i, rb).wait()


@jax.jit
def pallas_gated_mix__grouped_kv_mqa__swiglu_ffn__prompt_kernel(
    A_x, A_wq, A_wk, A_wv, A_wo, B_x, B_w_gate, B_w_up, B_w_down, gate_w
):
    hbm = pl.BlockSpec(memory_space=pl.ANY)
    vmem = pltpu.VMEM
    return pl.pallas_call(
        _kernel,
        grid=(NSTEP,),
        in_specs=[hbm] * 9,
        out_specs=hbm,
        out_shape=jax.ShapeDtypeStruct((1, S, D), bf16),
        scratch_shapes=[
            vmem((S, D), bf16),
            vmem((D, D), bf16),
            vmem((D,), bf16),
            vmem((2 * DH, D), bf16),
            vmem((S // 2, 128), u32),
            vmem((DH // 2, S), u32),
            vmem((D + DH, D), bf16),
            vmem((D // 2, TQ), u32),
            vmem((D, TQ), f32),
            vmem((D // 128, D, 128), bf16),
            vmem((F // 128, D, 128), bf16),
            vmem((F // 128, D, 128), bf16),
            vmem((D // 128, F, 128), bf16),
            vmem((DH, XVM, 128), f32),
            vmem((D, TQ), f32),
            vmem((8 * DH, TQ), f32),
            vmem((8 * DH, TQ), f32),
            vmem((XVM // 2, TQ), u32),
            vmem((XVM // 2, TQ), u32),
            vmem((TQ // 2, D), u32),
            vmem((TQ, D), f32),
            vmem((TQ, D), f32),
            vmem((S, TQ), f32),
            vmem((8, TQ), f32),
            vmem((TQ, 128), f32),
            vmem((8, TQ), f32),
            vmem((TQ, D), bf16),
            pltpu.SMEM((3,), f32),
            pltpu.SemaphoreType.DMA((NSEM,)),
        ],
        compiler_params=pltpu.CompilerParams(
            dimension_semantics=("arbitrary",), vmem_limit_bytes=100 * 1024 * 1024),
    )(A_x, A_wq, A_wk.T, A_wv.T, gate_w, A_wo, B_w_gate, B_w_up, B_w_down)
```

```python
import math

import jax
import jax.numpy as jnp
from jax import lax
from jax.experimental import pallas as pl
from jax.experimental.pallas import tpu as pltpu

S, D, H, DH, F = 2048, 512, 32, 16, 1792
TQ = 512
CK = 128
MB = 128
NCT = TQ // 128
NRB = TQ // MB
NSTEP = S // TQ
HPB = 4
NB = H // HPB - 1
FCH = F // NB
QSCALE = (DH ** -0.5) * math.log2(math.e)

S_MAX = 60.0
V_LO, V_HI = 2.0 ** -40, 2.0 ** 40

XV = 368
XV_LAST = [336, 352, 512]
XVM = max([XV] + XV_LAST)
LOOP_CFG = dict(gb=8, off=1, tsh=8, fpos=(1, 3, 6, 8, 11, -1), vpos=(10, -2))
LAST_CFG = dict(gb=8, off=2, tsh=0, fpos=(3, 8, -1), vpos=(9, -2), ext=150, ext_vpos=(8, 9, 10, 11))

X0 = 256
X0_FIRST, X0_SPARE = 4, 16

f32, bf16, u32 = jnp.float32, jnp.bfloat16, jnp.uint32
_NT = (((1,), (1,)), ((), ()))

SEM_WO = NB
SEM_X = NB + 1
SEM_SMALL = SEM_X + NSTEP
SEM_OUT = SEM_SMALL + 4
NSEM = SEM_OUT + NRB


def _kernel(x_hbm, wq_hbm, wkt_hbm, wvt_hbm, gw_hbm, wo_hbm, wg_hbm, wu_hbm, wd_hbm, o_hbm,
            x_ref, wq_ref, gw_ref, wkv_scr, k_scr, vt_scr, wqt_scr, qt_scr, ot_scr,
            wo_ref, wg_ref, wu_ref, wd_ref, kb_scr, qtf_scr, qb_a, qb_b, pv_a, pv_b, xq_scr,
            a_scr, b_scr, s_scr, lv_scr, g_scr, gt_scr, o_scr, stat, sems):
    i = pl.program_id(0)

    def mo(v, m):
        return v if isinstance(v, int) else pl.multiple_of(v, m)

    def chunk_copies(c):
        cps = []
        for f in range(2):
            col = mo(c * FCH + f * 128, 128)
            cps.append(pltpu.make_async_copy(wg_hbm.at[:, pl.ds(col, 128)], wg_ref.at[2 * c + f], sems.at[c]))
            cps.append(pltpu.make_async_copy(wu_hbm.at[:, pl.ds(col, 128)], wu_ref.at[2 * c + f], sems.at[c]))
        row = mo(c * FCH, FCH)
        for j in range(D // 128):
            cps.append(pltpu.make_async_copy(wd_hbm.at[pl.ds(row, FCH), pl.ds(j * 128, 128)],
                                             wd_ref.at[j, pl.ds(row, FCH), :], sems.at[c]))
        return cps

    def wo_copies():
        return [pltpu.make_async_copy(wo_hbm.at[:, pl.ds(j * 128, 128)], wo_ref.at[j], sems.at[SEM_WO])
                for j in range(D // 128)]

    def x_copy(c):
        return pltpu.make_async_copy(x_hbm.at[0, pl.ds(c * TQ, TQ), :], x_ref.at[pl.ds(c * TQ, TQ), :],
                                     sems.at[SEM_X + c])

    def small_copies():
        return [
            pltpu.make_async_copy(wkt_hbm, wkv_scr.at[pl.ds(0, DH), :], sems.at[SEM_SMALL]),
            pltpu.make_async_copy(wvt_hbm, wkv_scr.at[pl.ds(DH, DH), :], sems.at[SEM_SMALL + 1]),
            pltpu.make_async_copy(wq_hbm, wq_ref, sems.at[SEM_SMALL + 2]),
            pltpu.make_async_copy(gw_hbm, gw_ref, sems.at[SEM_SMALL + 3]),
        ]

    def out_copy(step, rb):
        return pltpu.make_async_copy(o_scr.at[pl.ds(rb * MB, MB), :],
                                     o_hbm.at[0, pl.ds(pl.multiple_of(step * TQ + rb * MB, MB), MB), :],
                                     sems.at[SEM_OUT + rb])

    def packed(ref, idx, r0, n):
        return pltpu.bitcast(ref.bitcast(u32)[idx, pl.ds(mo(r0 // 2, 8), n // 2), :], bf16)

    def packed_wide(ref, r0, n):
        return jnp.concatenate([packed(ref, j, r0, n) for j in range(D // 128)], axis=1)

    def kv_block(c):
        kvt = lax.dot_general(wkv_scr[...], x_ref[c * TQ:(c + 1) * TQ, :], _NT,
                              preferred_element_type=f32).astype(bf16)
        vt_scr[:, c * TQ:(c + 1) * TQ] = pltpu.bitcast(kvt[DH:2 * DH, :], u32)
        kvf = kvt.astype(f32)
        kt, vt = kvf[0:DH, :], kvf[DH:2 * DH, :]
        k2 = jnp.sum(kt * kt, axis=0, keepdims=True)
        vabs = jnp.abs(vt)
        krows = jnp.concatenate([kt, jnp.zeros((128 - DH, TQ), f32)], axis=0).T
        ku = pltpu.bitcast(krows.astype(bf16), u32)
        for t in range(TQ // CK):
            for g in range(8):
                r = (c * (TQ // CK) + t) * 64 + g * 8
                k_scr[r:r + 8, :] = ku[t * 64 + (7 - g) * 8:t * 64 + (7 - g) * 8 + 8, :]
        if c == 0:
            for d in range(DH):
                kb_scr[d] = jnp.broadcast_to(krows[:XVM, d:d + 1], (XVM, 128))
        return k2, vabs

    zeros = jnp.zeros((128 - DH, TQ), bf16)
    qbs = (qb_a, qb_b)
    pvs = (pv_a, pv_b)
    always = jnp.full((8, 128), i, jnp.int32) >= 0

    def qk_weights(h):
        return jnp.concatenate([pltpu.bitcast(qt_scr[pl.ds(mo(h * 8, 8), 8), :], bf16), zeros], axis=0)

    def fill_qb(h, par):
        qh = qtf_scr[pl.ds(mo(h * DH, DH), DH), :]
        for d in range(DH):
            qbs[par][8 * d:8 * d + 8, :] = jnp.broadcast_to(qh[d:d + 1, :], (8, TQ))

    def vt_tile(t):
        return pltpu.bitcast(vt_scr[:, t * CK:(t + 1) * CK], bf16)

    def exp_tile(s, l):
        n = s.shape[0] // 16
        p = jnp.exp2(s)
        for r in range(2 * n):
            pr = p[8 * r:8 * r + 8, :]
            l = pr if l is None else l + pr
        pt = jnp.concatenate([p[16 * (n - 1 - g):16 * (n - g), :] for g in range(n)], axis=0).astype(bf16)
        return pt, l

    def q_phase(row0, x0, late):
        qmax = None
        lv = [None] * NCT

        def vpu_tile(j, ticks):
            cols = slice(j * 128, (j + 1) * 128)
            nblk = x0 // 64
            for step in range(nblk * DH):
                bi, d = step // DH, step % DH
                tv, tr = ticks[(step * len(ticks)) // (nblk * DH)]
                qd = jnp.where(always, qb_a[8 * d:8 * d + 8, cols], tv[8 * tr:8 * tr + 8, 0:128])
                tt = kb_scr[d, bi * 64:(bi + 1) * 64, :].reshape(8, 8, 128) * qd[None]
                acc = tt if d == 0 else acc + tt
                if d == DH - 1:
                    ps = jnp.exp2(acc)
                    for g in range(8):
                        lv[j] = ps[g] if lv[j] is None else lv[j] + ps[g]
                    pv_a[bi * 32:(bi + 1) * 32, cols] = pltpu.bitcast(ps.reshape(64, 128).astype(bf16), u32)

        alltk = []
        ntk = NCT * (D + DH) // 8 + (XV - x0) // 8 + NRB * 16 - X0_FIRST - X0_SPARE
        done = [0]

        def emit(jmax):
            while done[0] <= jmax:
                j = done[0]
                lo, hi = X0_FIRST + (j * ntk) // NCT, X0_FIRST + ((j + 1) * ntk) // NCT
                if hi > len(alltk):
                    break
                vpu_tile(j, alltk[lo:hi])
                done[0] += 1

        for j in range(NCT):
            cols = slice(j * 128, (j + 1) * 128)
            xq = x_ref[pl.ds(mo(row0 + j * 128, 128), 128), :]
            xq_scr[j * 64:(j + 1) * 64, :] = pltpu.bitcast(xq, u32)
            qt = lax.dot_general(wqt_scr[...], xq, _NT, preferred_element_type=f32)
            gt = jax.nn.sigmoid(qt[D:D + 8, :])
            gt_scr[:, cols] = gt
            g_scr[cols, :] = jnp.concatenate([1.0 - gt] * 16, axis=0).T
            qtb = (qt[0:D, :] * QSCALE).astype(bf16)
            qt_scr[:, cols] = pltpu.bitcast(qtb, u32)
            qf = qtb.astype(f32)
            qtf_scr[:, cols] = qf
            q2 = qf * qf
            qn = None
            for h in range(H):
                t2 = q2[h * DH:h * DH + 8, :] + q2[h * DH + 8:(h + 1) * DH, :]
                qn = t2 if qn is None else jnp.maximum(qn, t2)
            qn = jnp.sum(qn, axis=0, keepdims=True)
            qmax = qn if qmax is None else jnp.maximum(qmax, qn)
            if x0:
                for d in range(DH):
                    qb_a[8 * d:8 * d + 8, cols] = jnp.broadcast_to(qf[d:d + 1, :], (8, 128))
                alltk += [(qt, r) for r in range((D + DH) // 8)]
                emit(j)
        stat[2] = jnp.max(qmax)
        if not x0:
            late()
        w0 = qk_weights(0)
        l0 = None
        tk = []
        k0 = x0
        while k0 < XV:
            t = k0 // CK
            k1 = min((t + 1) * CK, XV)
            r0 = t * 64 + ((t + 1) * CK - k1) // 2
            s0 = jnp.dot(pltpu.bitcast(k_scr[r0:r0 + (k1 - k0) // 2, :], bf16), w0, preferred_element_type=f32)
            pt, l0 = exp_tile(s0, l0)
            pv_a[k0 // 2:k1 // 2, :] = pltpu.bitcast(pt, u32)
            tk += [(s0, r) for r in range((k1 - k0) // 8)]
            k0 = k1
        if x0:
            alltk += tk
            emit(NCT - 1)
            for r in late():
                alltk += [(r, g) for g in range(16)]
            emit(NCT - 1)
            assert done[0] == NCT
            l0 = l0 + jnp.concatenate(lv, axis=1)
        lv_scr[...] = l0

    @pl.when(i == 0)
    def _():
        sm = small_copies()
        sm[2].start()
        x_copy(0).start()
        for cp in (sm[0], sm[1], sm[3]):
            cp.start()
        for c in range(1, NSTEP):
            x_copy(c).start()
        for cp in chunk_copies(0):
            cp.start()
        b_scr[...] = jnp.zeros_like(b_scr)
        sm[2].wait()
        wqt_scr[0:D, :] = wq_ref[...].astype(f32).T.astype(bf16)
        x_copy(0).wait()
        sm[0].wait()
        sm[1].wait()
        sm[3].wait()
        gw = jnp.broadcast_to(gw_ref[...].astype(f32).reshape(1, D), (DH, D))
        wqt_scr[D:D + DH, :] = gw.astype(bf16)
        k2_0, vabs_0 = kv_block(0)

        def rest_kv():
            k2, vabs = k2_0, vabs_0
            for c in range(1, NSTEP):
                x_copy(c).wait()
            for c in range(1, NB):
                for cp in chunk_copies(c):
                    cp.start()
            for cp in wo_copies():
                cp.start()
            for c in range(1, NSTEP):
                a, b = kv_block(c)
                k2 = jnp.maximum(k2, a)
                vabs = jnp.maximum(vabs, b)
            stat[0] = jnp.max(k2)
            vcol = jnp.max(vabs, axis=1, keepdims=True)
            v_ok = (vcol == 0.0) | ((vcol >= V_LO) & (vcol <= V_HI))
            stat[1] = jnp.min(jnp.where(v_ok, 1.0, 0.0))

        q_phase(0, 0, rest_kv)

    safe = jnp.logical_and(stat[2] * stat[0] <= S_MAX * S_MAX, stat[1] > 0.5)

    def finish(h, acc, l):
        lt = jnp.sum(l, axis=0, keepdims=True)
        ot_scr[pl.ds(mo(h * DH, DH), DH), :] = acc * (gt_scr[0:1, :] / lt)

    def x_rows(rb):
        return pltpu.bitcast(xq_scr[rb * MB // 2:(rb + 1) * MB // 2, :], bf16)

    def ffn_units(c):
        st = {}

        def gate(rb, f):
            def unit():
                g = jnp.dot(x_rows(rb), packed(wg_ref, 2 * c + f, 0, D), preferred_element_type=f32)
                hg = 0.5 * g
                st[rb, f] = hg + hg * jnp.tanh(hg)
                return g
            return unit

        def up(rb, f):
            def unit():
                u = jnp.dot(x_rows(rb), packed(wu_ref, 2 * c + f, 0, D), preferred_element_type=f32)
                st['act', rb, f] = (st.pop((rb, f)) * u).astype(bf16)
                return u
            return unit

        def down(rb, f):
            def unit():
                act = st.pop(('act', rb, f))
                r = jnp.dot(act, packed_wide(wd_ref, c * FCH + f * 128, 128), preferred_element_type=f32)
                b_scr[rb * MB:(rb + 1) * MB, :] += r
                return r
            return unit

        pieces = [(rb, f) for rb in range(NRB) for f in range(2)]
        units = []
        for n, (rb, f) in enumerate(pieces):
            units += [gate(rb, f), up(rb, f)]
            if n >= 1:
                units.append(down(*pieces[n - 1]))
        units.append(down(*pieces[-1]))
        return units

    def oproj_units():
        def make(kt, rb):
            def unit():
                rows = slice(rb * MB, (rb + 1) * MB)
                o = ot_scr[kt * 128:(kt + 1) * 128, rows].T.astype(bf16)
                r = jnp.dot(o, packed_wide(wo_ref, kt * 128, 128), preferred_element_type=f32)
                if kt == 1:
                    a_scr[rows, :] = r
                elif kt == 2:
                    a_scr[rows, :] += r
                else:
                    gm = jnp.concatenate([g_scr[rows, :]] * (D // 128), axis=1)
                    a_scr[rows, :] += r + gm * b_scr[rows, :]
                    b_scr[rows, :] = jnp.zeros((MB, D), f32)
                return r
            return unit
        return [make(kt, rb) for kt in (1, 2, 0) for rb in range(NRB)]

    def heads(h0, lv, units, xvs, gb, off, tsh, fpos, vpos, ext=0, ext_vpos=()):
        per_head = len(units) // HPB
        assert per_head == len(fpos)
        units = list(units)
        pend = None
        state = {}
        ticks = []
        prev = None
        for hr in range(HPB):
            par = hr % 2
            xv, xvn = xvs[hr], xvs[hr + 1]
            late = bool(ext) and hr == HPB - 1
            nvt = xv // CK
            nm = S // CK - nvt
            rows = [CK - (xv - nvt * CK)] + [CK] * (nm - 1)
            fslots = [v % nm for v in fpos]
            vslots = {(ext_vpos if late else vpos)[t] % nm: t for t in range(nvt)}
            ntick = sum(rows) // 8 + per_head * 16 + (ext if hr == HPB - 2 else 0)
            ng = xvn // 8
            nblk = -(-ng // gb)
            sched, cost = [], 0
            for bi in range(nblk):
                g0, g1 = 2 * ((bi * ng // 2) // nblk), 2 * (((bi + 1) * ng // 2) // nblk)
                for j in range(NCT):
                    for d in range(DH):
                        sched.append((g0, g1 - g0, j, d, cost))
                        cost += 2 * (g1 - g0) + 1 + (2 * (g1 - g0) if d == DH - 1 else 0)
            w = qk_weights(h0 + hr)
            if xvn:
                fill_qb(h0 + hr + 1, 1 - par)
            state[hr] = dict(acc=None, l=None if late else jnp.concatenate(lv, axis=1))
            vs = dict(todo=sched, acc=None, lvn=[None] * NCT)

            def vpu_steps(vs=vs, cost=cost, ntick=ntick, tick0=len(ticks) - tsh, par=par):
                while vs['todo'] and tick0 + (vs['todo'][0][4] * ntick) // cost < len(ticks):
                    g0, n, j, d, c0 = vs['todo'].pop(0)
                    tick = tick0 + (c0 * ntick) // cost
                    k0 = g0 * 8
                    qd = qbs[1 - par][8 * d:8 * d + 8, 128 * j:128 * (j + 1)]
                    if tick >= 0:
                        tv, tr = ticks[tick]
                        jj = j % (tv.shape[1] // 128)
                        qd = jnp.where(always, qd, tv[8 * tr:8 * tr + 8, 128 * jj:128 * (jj + 1)])
                    tt = kb_scr[d, k0:k0 + 8 * n, :].reshape(n, 8, 128) * qd[None]
                    vs['acc'] = tt if d == 0 else vs['acc'] + tt
                    if d == DH - 1:
                        ps = jnp.exp2(vs['acc'])
                        for g in range(n):
                            vs['lvn'][j] = ps[g] if vs['lvn'][j] is None else vs['lvn'][j] + ps[g]
                        pc = ps.reshape(8 * n, 128).astype(bf16)
                        pvs[1 - par][k0 // 2:k0 // 2 + 4 * n, 128 * j:128 * (j + 1)] = pltpu.bitcast(pc, u32)

            def advance(val):
                for r in range(val.shape[0] // 8):
                    ticks.append((val, r))
                if late:
                    prev[0]()
                vpu_steps()

            def add_pv(st, tile_idx, p_tile):
                o = jnp.dot(vt_tile(tile_idx), p_tile, preferred_element_type=f32)
                st['acc'] = o if st['acc'] is None else st['acc'] + o

            stream = [(nvt + c, g) for c in range(nm) for g in range(rows[c] // 16)]
            bounds = [0] + [min(sum(rows[:c + 1]) // 16 + off, len(stream)) for c in range(nm)]
            parts = {}
            for c in range(nm):
                grp = stream[bounds[c]:bounds[c + 1]]
                runs = []
                for (t, g) in grp:
                    r = t * 64 + g * 8
                    if runs and runs[-1][1] == r:
                        runs[-1][1] = r + 8
                    else:
                        runs.append([r, r + 8])
                lhs = [k_scr[r0:r1, :] for r0, r1 in runs]
                lhs = lhs[0] if len(lhs) == 1 else jnp.concatenate(lhs, axis=0)
                s = jnp.dot(pltpu.bitcast(lhs, bf16), w, preferred_element_type=f32)
                if c in vslots:
                    tv = vslots[c]
                    assert prev is None or all(st[0] * 8 >= (tv + 1) * CK for st in prev[1]['todo'])
                    add_pv(state[hr], tv, pltpu.bitcast(pvs[par][tv * 64:(tv + 1) * 64, :], bf16))
                if pend is not None:
                    ph, ppt, ptile, plast = pend
                    add_pv(state[ph], ptile, ppt)
                    if plast:
                        finish(h0 + ph, state[ph]['acc'], state[ph]['l'])
                p = jnp.exp2(s)
                for n, (t, g) in enumerate(grp):
                    for r in (2 * n, 2 * n + 1):
                        pr = p[8 * r:8 * r + 8, :]
                        state[hr]['l'] = pr if state[hr]['l'] is None else state[hr]['l'] + pr
                    parts.setdefault(t, []).append(p[16 * n:16 * n + 16, :])
                t = nvt + c
                tile = jnp.concatenate(parts.pop(t)[::-1], axis=0).astype(bf16)
                if rows[c] < CK:
                    assert not late
                    nvr = CK - rows[c]
                    tile = jnp.concatenate([pltpu.bitcast(pvs[par][t * 64:t * 64 + nvr // 2, :], bf16), tile], axis=0)
                pend = (hr, tile, t, c == nm - 1)
                advance(s)
                for _ in range(fslots.count(c)):
                    advance(units.pop(0)())
            assert not vs['todo'] or (ext and hr == HPB - 2)
            if late:
                assert not prev[1]['todo']
                state[hr]['l'] = state[hr]['l'] + jnp.concatenate(lv, axis=1)
            lv = vs['lvn']
            prev = (vpu_steps, vs)
        assert not units
        ph, ppt, ptile, _ = pend
        o = jnp.dot(vt_tile(ptile), ppt, preferred_element_type=f32)
        finish(h0 + ph, state[ph]['acc'] + o, state[ph]['l'])
        return lv

    def wait_first(copies):
        @pl.when(i == 0)
        def _():
            for cp in copies:
                cp.wait()

    @pl.when(safe)
    def _fast():
        lv0 = [lv_scr[:, 128 * j:128 * (j + 1)] for j in range(NCT)]

        def body(it, lv):
            wait_first(chunk_copies(it))
            return heads(it * HPB, lv, ffn_units(it), [XV] * (HPB + 1), **LOOP_CFG)

        lv = lax.fori_loop(0, NB, body, lv0)
        wait_first(wo_copies())
        heads(NB * HPB, lv, oproj_units(), [XV] + XV_LAST + [0], **LAST_CFG)

    @pl.when(jnp.logical_not(safe))
    def _exact():
        def head(h, carry):
            w = qk_weights(h)
            m = None
            for t in range(S // CK):
                sc = jnp.dot(pltpu.bitcast(k_scr[t * 64:(t + 1) * 64, :], bf16), w, preferred_element_type=f32)
                s_scr[t * CK:(t + 1) * CK, :] = sc
                for r in range(CK // 8):
                    sr = sc[8 * r:8 * r + 8, :]
                    m = sr if m is None else jnp.maximum(m, sr)
            m = jnp.max(m, axis=0, keepdims=True)
            l = acc = None
            for t in range(S // CK):
                pt, l = exp_tile(s_scr[t * CK:(t + 1) * CK, :] - m, l)
                o = jnp.dot(vt_tile(t), pt, preferred_element_type=f32)
                acc = o if acc is None else acc + o
            finish(h, acc, l)
            return carry

        lax.fori_loop(0, H, head, 0)

        def ffn(it, carry):
            wait_first(chunk_copies(it))
            for unit in ffn_units(it):
                unit()
            return carry

        lax.fori_loop(0, NB, ffn, 0)
        wait_first(wo_copies())
        for unit in oproj_units():
            unit()

    def tail():
        res = []
        for rb in range(NRB):
            rows = slice(rb * MB, (rb + 1) * MB)
            o = ot_scr[3 * 128:4 * 128, rows].T.astype(bf16)
            r = jnp.dot(o, packed_wide(wo_ref, 3 * 128, 128), preferred_element_type=f32)
            o_scr[rows, :] = (a_scr[rows, :] + r).astype(bf16)
            out_copy(i, rb).start()
            res.append(r)
        return res

    @pl.when(i > 0)
    def _():
        for rb in range(NRB):
            out_copy(i - 1, rb).wait()

    @pl.when(i < NSTEP - 1)
    def _():
        q_phase((i + 1) * TQ, X0, tail)

    @pl.when(i == NSTEP - 1)
    def _():
        tail()
        for rb in range(NRB):
            out_copy(i, rb).wait()


@jax.jit
def pallas_gated_mix__grouped_kv_mqa__swiglu_ffn__prompt_kernel(
    A_x, A_wq, A_wk, A_wv, A_wo, B_x, B_w_gate, B_w_up, B_w_down, gate_w
):
    hbm = pl.BlockSpec(memory_space=pl.ANY)
    vmem = pltpu.VMEM
    return pl.pallas_call(
        _kernel,
        grid=(NSTEP,),
        in_specs=[hbm] * 9,
        out_specs=hbm,
        out_shape=jax.ShapeDtypeStruct((1, S, D), bf16),
        scratch_shapes=[
            vmem((S, D), bf16),
            vmem((D, D), bf16),
            vmem((D,), bf16),
            vmem((2 * DH, D), bf16),
            vmem((S // 2, 128), u32),
            vmem((DH // 2, S), u32),
            vmem((D + DH, D), bf16),
            vmem((D // 2, TQ), u32),
            vmem((D, TQ), f32),
            vmem((D // 128, D, 128), bf16),
            vmem((F // 128, D, 128), bf16),
            vmem((F // 128, D, 128), bf16),
            vmem((D // 128, F, 128), bf16),
            vmem((DH, XVM, 128), f32),
            vmem((D, TQ), f32),
            vmem((8 * DH, TQ), f32),
            vmem((8 * DH, TQ), f32),
            vmem((XVM // 2, TQ), u32),
            vmem((XVM // 2, TQ), u32),
            vmem((TQ // 2, D), u32),
            vmem((TQ, D), f32),
            vmem((TQ, D), f32),
            vmem((S, TQ), f32),
            vmem((8, TQ), f32),
            vmem((TQ, 128), f32),
            vmem((8, TQ), f32),
            vmem((TQ, D), bf16),
            pltpu.SMEM((3,), f32),
            pltpu.SemaphoreType.DMA((NSEM,)),
        ],
        compiler_params=pltpu.CompilerParams(
            dimension_semantics=("arbitrary",), vmem_limit_bytes=100 * 1024 * 1024),
    )(A_x, A_wq, A_wk.T, A_wv.T, gate_w, A_wo, B_w_gate, B_w_up, B_w_down)
```

```python
import math

import jax
import jax.numpy as jnp
from jax import lax
from jax.experimental import pallas as pl
from jax.experimental.pallas import tpu as pltpu

S, D, H, DH, F = 2048, 512, 32, 16, 1792
TQ = 512
CK = 128
MB = 128
NCT = TQ // 128
NRB = TQ // MB
NSTEP = S // TQ
HPB = 4
NB = H // HPB - 1
FCH = F // NB
QSCALE = (DH ** -0.5) * math.log2(math.e)

S_MAX = 60.0
V_LO, V_HI = 2.0 ** -40, 2.0 ** 40

XV_LOOP = [368, 352, 368, 368]
XV = XV_LOOP[0]
XV_LAST = [352, 336, 512]
XVM = max(XV_LOOP + XV_LAST)
LOOP_CFG = dict(gb=8, off=1, tsh=9, fpos=(1, 3, 6, 8, 11, -1), vpos=(7, -2))
LAST_CFG = dict(gb=8, off=2, tsh=6, fpos=(3, 8, -1), vpos=(7, -2), ext=160, ext_vpos=(6, 9, 10, 11))
X0 = 320
X0_FIRST, X0_SPARE = 3, 8

f32, bf16, u32 = jnp.float32, jnp.bfloat16, jnp.uint32
_NT = (((1,), (1,)), ((), ()))

SEM_WO = NB
SEM_X = NB + 1
SEM_SMALL = SEM_X + NSTEP
SEM_OUT = SEM_SMALL + 4
NSEM = SEM_OUT + NRB


def _kernel(x_hbm, wq_hbm, wkt_hbm, wvt_hbm, gw_hbm, wo_hbm, wg_hbm, wu_hbm, wd_hbm, o_hbm,
            x_ref, wq_ref, gw_ref, wkv_scr, k_scr, vt_scr, wqt_scr, qt_scr, ot_scr,
            wo_ref, wg_ref, wu_ref, wd_ref, kb_scr, qtf_scr, qb_a, qb_b, pv_a, pv_b, xq_scr,
            a_scr, b_scr, s_scr, lv_scr, g_scr, gt_scr, o_scr, stat, sems):
    i = pl.program_id(0)

    def mo(v, m):
        return v if isinstance(v, int) else pl.multiple_of(v, m)

    def chunk_copies(c):
        cps = []
        for f in range(2):
            col = mo(c * FCH + f * 128, 128)
            cps.append(pltpu.make_async_copy(wg_hbm.at[:, pl.ds(col, 128)], wg_ref.at[2 * c + f], sems.at[c]))
            cps.append(pltpu.make_async_copy(wu_hbm.at[:, pl.ds(col, 128)], wu_ref.at[2 * c + f], sems.at[c]))
        row = mo(c * FCH, FCH)
        for j in range(D // 128):
            cps.append(pltpu.make_async_copy(wd_hbm.at[pl.ds(row, FCH), pl.ds(j * 128, 128)],
                                             wd_ref.at[j, pl.ds(row, FCH), :], sems.at[c]))
        return cps

    def wo_copies():
        return [pltpu.make_async_copy(wo_hbm.at[:, pl.ds(j * 128, 128)], wo_ref.at[j], sems.at[SEM_WO])
                for j in range(D // 128)]

    def x_copy(c):
        return pltpu.make_async_copy(x_hbm.at[0, pl.ds(c * TQ, TQ), :], x_ref.at[pl.ds(c * TQ, TQ), :],
                                     sems.at[SEM_X + c])

    def small_copies():
        return [
            pltpu.make_async_copy(wkt_hbm, wkv_scr.at[pl.ds(0, DH), :], sems.at[SEM_SMALL]),
            pltpu.make_async_copy(wvt_hbm, wkv_scr.at[pl.ds(DH, DH), :], sems.at[SEM_SMALL + 1]),
            pltpu.make_async_copy(wq_hbm, wq_ref, sems.at[SEM_SMALL + 2]),
            pltpu.make_async_copy(gw_hbm, gw_ref, sems.at[SEM_SMALL + 3]),
        ]

    def out_copy(step, rb):
        return pltpu.make_async_copy(o_scr.at[pl.ds(rb * MB, MB), :],
                                     o_hbm.at[0, pl.ds(pl.multiple_of(step * TQ + rb * MB, MB), MB), :],
                                     sems.at[SEM_OUT + rb])

    def wide(ref, r0):
        return jnp.concatenate([ref[j, pl.ds(mo(r0, 128), 128), :] for j in range(D // 128)], axis=1)

    def kv_block(c):
        kvt = lax.dot_general(wkv_scr[...], x_ref[c * TQ:(c + 1) * TQ, :], _NT,
                              preferred_element_type=f32).astype(bf16)
        vt_scr[:, c * TQ:(c + 1) * TQ] = pltpu.bitcast(kvt[DH:2 * DH, :], u32)
        kvf = kvt.astype(f32)
        kt, vt = kvf[0:DH, :], kvf[DH:2 * DH, :]
        k2 = jnp.sum(kt * kt, axis=0, keepdims=True)
        vabs = jnp.abs(vt)
        krows = jnp.concatenate([kt, jnp.zeros((128 - DH, TQ), f32)], axis=0).T
        ku = pltpu.bitcast(krows.astype(bf16), u32)
        for t in range(TQ // CK):
            for g in range(8):
                r = (c * (TQ // CK) + t) * 64 + g * 8
                k_scr[r:r + 8, :] = ku[t * 64 + (7 - g) * 8:t * 64 + (7 - g) * 8 + 8, :]
        if c == 0:
            for d in range(DH):
                kb_scr[d] = jnp.broadcast_to(krows[:XVM, d:d + 1], (XVM, 128))
        return k2, vabs

    zeros = jnp.zeros((128 - DH, TQ), bf16)
    qbs = (qb_a, qb_b)
    pvs = (pv_a, pv_b)
    always = jnp.full((8, 128), i, jnp.int32) >= 0

    def qk_weights(h):
        return jnp.concatenate([pltpu.bitcast(qt_scr[pl.ds(mo(h * 8, 8), 8), :], bf16), zeros], axis=0)

    def fill_qb(h, par):
        qh = qtf_scr[pl.ds(mo(h * DH, DH), DH), :]
        qbs[par][...] = jnp.concatenate([jnp.broadcast_to(qh[d:d + 1, :], (8, TQ)) for d in range(DH)], axis=0)

    def vt_tile(t):
        return pltpu.bitcast(vt_scr[:, t * CK:(t + 1) * CK], bf16)

    def exp_tile(s, l):
        n = s.shape[0] // 16
        p = jnp.exp2(s)
        for r in range(2 * n):
            pr = p[8 * r:8 * r + 8, :]
            l = pr if l is None else l + pr
        pt = jnp.concatenate([p[16 * (n - 1 - g):16 * (n - g), :] for g in range(n)], axis=0).astype(bf16)
        return pt, l

    def q_phase(row0, x0, late):
        qmax = None
        lv = [None] * NCT

        def vpu_tile(j, ticks):
            cols = slice(j * 128, (j + 1) * 128)
            nblk = x0 // 64
            for step in range(nblk * DH):
                bi, d = step // DH, step % DH
                tv, tr = ticks[(step * len(ticks)) // (nblk * DH)]
                if d == 0:
                    qall, kall = qb_a[:, cols], kb_scr[:, bi * 64:(bi + 1) * 64, :]
                qd = jnp.where(always, qall[8 * d:8 * d + 8, :], tv[8 * tr:8 * tr + 8, 0:128])
                tt = kall[d].reshape(8, 8, 128) * qd[None]
                acc = tt if d == 0 else acc + tt
                if d == DH - 1:
                    ps = jnp.exp2(acc)
                    for g in range(8):
                        lv[j] = ps[g] if lv[j] is None else lv[j] + ps[g]
                    pv_a[bi * 32:(bi + 1) * 32, cols] = pltpu.bitcast(ps.reshape(64, 128).astype(bf16), u32)

        alltk = []
        ntk = NCT * (D + DH) // 8 + (XV - x0) // 8 + NRB * 16 - X0_FIRST - X0_SPARE
        done = [0]

        def emit(jmax):
            while done[0] <= jmax:
                j = done[0]
                lo, hi = X0_FIRST + (j * ntk) // NCT, X0_FIRST + ((j + 1) * ntk) // NCT
                if hi > len(alltk):
                    break
                vpu_tile(j, alltk[lo:hi])
                done[0] += 1

        for j in range(NCT):
            cols = slice(j * 128, (j + 1) * 128)
            xq = x_ref[pl.ds(mo(row0 + j * 128, 128), 128), :]
            xq_scr[j * 64:(j + 1) * 64, :] = pltpu.bitcast(xq, u32)
            qt = lax.dot_general(pltpu.bitcast(wqt_scr[...], bf16), xq, _NT, preferred_element_type=f32)
            gt = jax.nn.sigmoid(qt[D:D + 8, :])
            gt_scr[:, cols] = gt
            g_scr[cols, :] = jnp.concatenate([1.0 - gt] * 16, axis=0).T
            qtb = (qt[0:D, :] * QSCALE).astype(bf16)
            qt_scr[:, cols] = pltpu.bitcast(qtb, u32)
            qf = qtb.astype(f32)
            qtf_scr[:, cols] = qf
            q2 = qf * qf
            qn = None
            for h in range(H):
                t2 = q2[h * DH:h * DH + 8, :] + q2[h * DH + 8:(h + 1) * DH, :]
                qn = t2 if qn is None else jnp.maximum(qn, t2)
            qn = jnp.sum(qn, axis=0, keepdims=True)
            qmax = qn if qmax is None else jnp.maximum(qmax, qn)
            if x0:
                for d in range(DH):
                    qb_a[8 * d:8 * d + 8, cols] = jnp.broadcast_to(qf[d:d + 1, :], (8, 128))
                alltk += [(qt, r) for r in range((D + DH) // 8)]
                emit(j)
        stat[2] = jnp.max(qmax)
        if not x0:
            late()
        w0 = qk_weights(0)
        l0 = None
        tk = []
        k0 = x0
        while k0 < XV:
            t = k0 // CK
            k1 = min((t + 1) * CK, XV)
            r0 = t * 64 + ((t + 1) * CK - k1) // 2
            s0 = jnp.dot(pltpu.bitcast(k_scr[r0:r0 + (k1 - k0) // 2, :], bf16), w0, preferred_element_type=f32)
            pt, l0 = exp_tile(s0, l0)
            pv_a[k0 // 2:k1 // 2, :] = pltpu.bitcast(pt, u32)
            tk += [(s0, r) for r in range((k1 - k0) // 8)]
            k0 = k1
        if x0:
            alltk += tk
            emit(NCT - 1)
            for r in late():
                alltk += [(r, g) for g in range(16)]
            emit(NCT - 1)
            assert done[0] == NCT
            l0 = l0 + jnp.concatenate(lv, axis=1)
        lv_scr[...] = l0

    @pl.when(i == 0)
    def _():
        sm = small_copies()
        sm[2].start()
        x_copy(0).start()
        for cp in (sm[0], sm[1], sm[3]):
            cp.start()
        for c in range(1, NSTEP):
            x_copy(c).start()
        for cp in chunk_copies(0):
            cp.start()
        b_scr[...] = jnp.zeros_like(b_scr)
        sm[2].wait()
        wqt_scr[0:D // 2, :] = pltpu.bitcast(wq_ref[...].astype(f32).T.astype(bf16), u32)
        x_copy(0).wait()
        sm[0].wait()
        sm[1].wait()
        sm[3].wait()
        gw = jnp.broadcast_to(gw_ref[...].astype(f32).reshape(1, D), (DH, D))
        wqt_scr[D // 2:(D + DH) // 2, :] = pltpu.bitcast(gw.astype(bf16), u32)
        k2_0, vabs_0 = kv_block(0)

        def rest_kv():
            k2, vabs = k2_0, vabs_0
            for c in range(1, NSTEP):
                x_copy(c).wait()
            for c in range(1, NB):
                for cp in chunk_copies(c):
                    cp.start()
            for cp in wo_copies():
                cp.start()
            for c in range(1, NSTEP):
                a, b = kv_block(c)
                k2 = jnp.maximum(k2, a)
                vabs = jnp.maximum(vabs, b)
            stat[0] = jnp.max(k2)
            vcol = jnp.max(vabs, axis=1, keepdims=True)
            v_ok = (vcol == 0.0) | ((vcol >= V_LO) & (vcol <= V_HI))
            stat[1] = jnp.min(jnp.where(v_ok, 1.0, 0.0))

        q_phase(0, 0, rest_kv)

    safe = jnp.logical_and(stat[2] * stat[0] <= S_MAX * S_MAX, stat[1] > 0.5)

    def finish(h, acc, l):
        lt = jnp.sum(l, axis=0, keepdims=True)
        ot_scr[pl.ds(mo(h * DH, DH), DH), :] = acc * (gt_scr[0:1, :] / lt)

    def x_rows(rb):
        return pltpu.bitcast(xq_scr[rb * MB // 2:(rb + 1) * MB // 2, :], bf16)

    def ffn_units(c):
        st = {}

        def gate(rb, f):
            def unit():
                g = jnp.dot(x_rows(rb), wg_ref[2 * c + f], preferred_element_type=f32)
                hg = 0.5 * g
                st[rb, f] = hg + hg * jnp.tanh(hg)
                return g
            return unit

        def up(rb, f):
            def unit():
                u = jnp.dot(x_rows(rb), wu_ref[2 * c + f], preferred_element_type=f32)
                st['act', rb, f] = (st.pop((rb, f)) * u).astype(bf16)
                return u
            return unit

        def down(rb, f):
            def unit():
                act = st.pop(('act', rb, f))
                r = jnp.dot(act, wide(wd_ref, c * FCH + f * 128), preferred_element_type=f32)
                b_scr[rb * MB:(rb + 1) * MB, :] += r
                return r
            return unit

        pieces = [(rb, f) for rb in range(NRB) for f in range(2)]
        units = []
        for n, (rb, f) in enumerate(pieces):
            units += [gate(rb, f), up(rb, f)]
            if n >= 1:
                units.append(down(*pieces[n - 1]))
        units.append(down(*pieces[-1]))
        return units

    def oproj_units():
        def make(kt, rb):
            def unit():
                rows = slice(rb * MB, (rb + 1) * MB)
                o = ot_scr[kt * 128:(kt + 1) * 128, rows].T.astype(bf16)
                r = jnp.dot(o, wide(wo_ref, kt * 128), preferred_element_type=f32)
                if kt == 1:
                    a_scr[rows, :] = r
                elif kt == 2:
                    a_scr[rows, :] += r
                else:
                    gm = jnp.concatenate([g_scr[rows, :]] * (D // 128), axis=1)
                    a_scr[rows, :] += r + gm * b_scr[rows, :]
                    b_scr[rows, :] = jnp.zeros((MB, D), f32)
                return r
            return unit
        return [make(kt, rb) for kt in (1, 2, 0) for rb in range(NRB)]

    def heads(h0, lv, units, xvs, gb, off, tsh, fpos, vpos, ext=0, ext_vpos=()):
        per_head = len(units) // HPB
        assert per_head == len(fpos)
        units = list(units)
        pend = None
        state = {}
        ticks = []
        prev = None
        for hr in range(HPB):
            par = hr % 2
            xv, xvn = xvs[hr], xvs[hr + 1]
            late = bool(ext) and hr == HPB - 1
            nvt = xv // CK
            nm = S // CK - nvt
            rows = [CK - (xv - nvt * CK)] + [CK] * (nm - 1)
            fslots = [v % nm for v in fpos]
            vslots = {(ext_vpos if late else vpos)[t] % nm: t for t in range(nvt)}
            ntick = sum(rows) // 8 + per_head * 16 + (ext if hr == HPB - 2 else 0)
            ng = xvn // 8
            nblk = -(-ng // gb)
            sched, cost = [], 0
            for bi in range(nblk):
                g0, g1 = 2 * ((bi * ng // 2) // nblk), 2 * (((bi + 1) * ng // 2) // nblk)
                for j in range(NCT):
                    for d in range(DH):
                        sched.append((g0, g1 - g0, j, d, cost))
                        cost += 2 * (g1 - g0) + 1 + (2 * (g1 - g0) if d == DH - 1 else 0)
            w = qk_weights(h0 + hr)
            if xvn:
                fill_qb(h0 + hr + 1, 1 - par)
            state[hr] = dict(acc=None, l=None if late else jnp.concatenate(lv, axis=1))
            vs = dict(todo=sched, acc=None, lvn=[None] * NCT)

            def vpu_steps(vs=vs, cost=cost, ntick=ntick, tick0=len(ticks) - tsh, par=par):
                while vs['todo'] and tick0 + (vs['todo'][0][4] * ntick) // cost < len(ticks):
                    g0, n, j, d, c0 = vs['todo'].pop(0)
                    tick = tick0 + (c0 * ntick) // cost
                    k0 = g0 * 8
                    if d == 0:
                        vs['q'] = qbs[1 - par][:, 128 * j:128 * (j + 1)]
                        vs['k'] = kb_scr[:, k0:k0 + 8 * n, :]
                    qd = vs['q'][8 * d:8 * d + 8, :]
                    if tick >= 0:
                        tv, tr = ticks[tick]
                        qd = jnp.where(always, qd, tv[8 * tr:8 * tr + 8, 0:128])
                    tt = vs['k'][d].reshape(n, 8, 128) * qd[None]
                    vs['acc'] = tt if d == 0 else vs['acc'] + tt
                    if d == DH - 1:
                        ps = jnp.exp2(vs['acc'])
                        for g in range(n):
                            vs['lvn'][j] = ps[g] if vs['lvn'][j] is None else vs['lvn'][j] + ps[g]
                        pc = ps.reshape(8 * n, 128).astype(bf16)
                        pvs[1 - par][k0 // 2:k0 // 2 + 4 * n, 128 * j:128 * (j + 1)] = pltpu.bitcast(pc, u32)

            def advance(val):
                for r in range(val.shape[0] // 8):
                    ticks.append((val, r))
                if late:
                    prev[0]()
                vpu_steps()

            def add_pv(st, tile_idx, p_tile):
                o = jnp.dot(vt_tile(tile_idx), p_tile, preferred_element_type=f32)
                st['acc'] = o if st['acc'] is None else st['acc'] + o

            stream = [(nvt + c, g) for c in range(nm) for g in range(rows[c] // 16)]
            bounds = [0] + [min(sum(rows[:c + 1]) // 16 + off, len(stream)) for c in range(nm)]
            parts = {}
            for c in range(nm):
                grp = stream[bounds[c]:bounds[c + 1]]
                runs = []
                for (t, g) in grp:
                    r = t * 64 + g * 8
                    if runs and runs[-1][1] == r:
                        runs[-1][1] = r + 8
                    else:
                        runs.append([r, r + 8])
                lhs = [k_scr[r0:r1, :] for r0, r1 in runs]
                lhs = lhs[0] if len(lhs) == 1 else jnp.concatenate(lhs, axis=0)
                s = jnp.dot(pltpu.bitcast(lhs, bf16), w, preferred_element_type=f32)
                if c in vslots:
                    tv = vslots[c]
                    assert prev is None or all(st[0] * 8 >= (tv + 1) * CK for st in prev[1]['todo'])
                    add_pv(state[hr], tv, pltpu.bitcast(pvs[par][tv * 64:(tv + 1) * 64, :], bf16))
                if pend is not None:
                    ph, ppt, ptile, plast = pend
                    add_pv(state[ph], ptile, ppt)
                    if plast:
                        finish(h0 + ph, state[ph]['acc'], state[ph]['l'])
                p = jnp.exp2(s)
                for n, (t, g) in enumerate(grp):
                    for r in (2 * n, 2 * n + 1):
                        pr = p[8 * r:8 * r + 8, :]
                        state[hr]['l'] = pr if state[hr]['l'] is None else state[hr]['l'] + pr
                    parts.setdefault(t, []).append(p[16 * n:16 * n + 16, :])
                t = nvt + c
                tile = jnp.concatenate(parts.pop(t)[::-1], axis=0).astype(bf16)
                if rows[c] < CK:
                    assert not late
                    nvr = CK - rows[c]
                    tile = jnp.concatenate([pltpu.bitcast(pvs[par][t * 64:t * 64 + nvr // 2, :], bf16), tile], axis=0)
                pend = (hr, tile, t, c == nm - 1)
                advance(s)
                for _ in range(fslots.count(c)):
                    advance(units.pop(0)())
            assert not vs['todo'] or (ext and hr == HPB - 2)
            if late:
                assert not prev[1]['todo']
                state[hr]['l'] = state[hr]['l'] + jnp.concatenate(lv, axis=1)
            lv = vs['lvn']
            prev = (vpu_steps, vs)
        assert not units
        ph, ppt, ptile, _ = pend
        o = jnp.dot(vt_tile(ptile), ppt, preferred_element_type=f32)
        finish(h0 + ph, state[ph]['acc'] + o, state[ph]['l'])
        return lv

    def wait_first(copies):
        @pl.when(i == 0)
        def _():
            for cp in copies:
                cp.wait()

    @pl.when(safe)
    def _fast():
        lv0 = [lv_scr[:, 128 * j:128 * (j + 1)] for j in range(NCT)]

        def body(it, lv):
            wait_first(chunk_copies(it))
            return heads(it * HPB, lv, ffn_units(it), XV_LOOP + [XV], **LOOP_CFG)

        lv = lax.fori_loop(0, NB, body, lv0)
        wait_first(wo_copies())
        heads(NB * HPB, lv, oproj_units(), [XV] + XV_LAST + [0], **LAST_CFG)

    @pl.when(jnp.logical_not(safe))
    def _exact():
        def head(h, carry):
            w = qk_weights(h)
            m = None
            for t in range(S // CK):
                sc = jnp.dot(pltpu.bitcast(k_scr[t * 64:(t + 1) * 64, :], bf16), w, preferred_element_type=f32)
                s_scr[t * CK:(t + 1) * CK, :] = sc
                for r in range(CK // 8):
                    sr = sc[8 * r:8 * r + 8, :]
                    m = sr if m is None else jnp.maximum(m, sr)
            m = jnp.max(m, axis=0, keepdims=True)
            l = acc = None
            for t in range(S // CK):
                pt, l = exp_tile(s_scr[t * CK:(t + 1) * CK, :] - m, l)
                o = jnp.dot(vt_tile(t), pt, preferred_element_type=f32)
                acc = o if acc is None else acc + o
            finish(h, acc, l)
            return carry

        lax.fori_loop(0, H, head, 0)

        def ffn(it, carry):
            wait_first(chunk_copies(it))
            for unit in ffn_units(it):
                unit()
            return carry

        lax.fori_loop(0, NB, ffn, 0)
        wait_first(wo_copies())
        for unit in oproj_units():
            unit()

    def tail():
        res = []
        for rb in range(NRB):
            rows = slice(rb * MB, (rb + 1) * MB)
            o = ot_scr[3 * 128:4 * 128, rows].T.astype(bf16)
            r = jnp.dot(o, wide(wo_ref, 3 * 128), preferred_element_type=f32)
            o_scr[rows, :] = (a_scr[rows, :] + r).astype(bf16)
            out_copy(i, rb).start()
            res.append(r)
        return res

    @pl.when(i > 0)
    def _():
        for rb in range(NRB):
            out_copy(i - 1, rb).wait()

    @pl.when(i < NSTEP - 1)
    def _():
        q_phase((i + 1) * TQ, X0, tail)

    @pl.when(i == NSTEP - 1)
    def _():
        tail()
        for rb in range(NRB):
            out_copy(i, rb).wait()


@jax.jit
def pallas_gated_mix__grouped_kv_mqa__swiglu_ffn__prompt_kernel(
    A_x, A_wq, A_wk, A_wv, A_wo, B_x, B_w_gate, B_w_up, B_w_down, gate_w
):
    hbm = pl.BlockSpec(memory_space=pl.ANY)
    vmem = pltpu.VMEM
    return pl.pallas_call(
        _kernel,
        grid=(NSTEP,),
        in_specs=[hbm] * 9,
        out_specs=hbm,
        out_shape=jax.ShapeDtypeStruct((1, S, D), bf16),
        scratch_shapes=[
            vmem((S, D), bf16),
            vmem((D, D), bf16),
            vmem((D,), bf16),
            vmem((2 * DH, D), bf16),
            vmem((S // 2, 128), u32),
            vmem((DH // 2, S), u32),
            vmem(((D + DH) // 2, D), u32),
            vmem((D // 2, TQ), u32),
            vmem((D, TQ), f32),
            vmem((D // 128, D, 128), bf16),
            vmem((F // 128, D, 128), bf16),
            vmem((F // 128, D, 128), bf16),
            vmem((D // 128, F, 128), bf16),
            vmem((DH, XVM, 128), f32),
            vmem((D, TQ), f32),
            vmem((8 * DH, TQ), f32),
            vmem((8 * DH, TQ), f32),
            vmem((XVM // 2, TQ), u32),
            vmem((XVM // 2, TQ), u32),
            vmem((TQ // 2, D), u32),
            vmem((TQ, D), f32),
            vmem((TQ, D), f32),
            vmem((S, TQ), f32),
            vmem((8, TQ), f32),
            vmem((TQ, 128), f32),
            vmem((8, TQ), f32),
            vmem((TQ, D), bf16),
            pltpu.SMEM((3,), f32),
            pltpu.SemaphoreType.DMA((NSEM,)),
        ],
        compiler_params=pltpu.CompilerParams(
            dimension_semantics=("arbitrary",), vmem_limit_bytes=100 * 1024 * 1024),
    )(A_x, A_wq, A_wk.T, A_wv.T, gate_w, A_wo, B_w_gate, B_w_up, B_w_down)
```
